```python
import os as _os
_os.environ.setdefault('JAX_PLATFORMS', 'cpu')
import jax
import jax.numpy as jnp

def _softmax(x, axis=-1):
    return jax.nn.softmax(x, axis=axis)

def _gelu(x):
    return jax.nn.gelu(x, approximate=True)

def _silu(x):
    return jax.nn.silu(x)

def _sigmoid(x):
    return jax.nn.sigmoid(x)

def _layernorm(x, axis=-1, eps=1e-05):
    m = jnp.mean(x, axis=axis, keepdims=True)
    v = jnp.var(x, axis=axis, keepdims=True)
    return (x - m) / jnp.sqrt(v + eps)

def _scatter_add(tgt, idx, src, axis=0):
    return tgt.at[idx].add(src)

def _segment_sum(src, seg, n):
    return jax.ops.segment_sum(src, seg, n)

class _Rng:

    def __init__(self, key):
        self._k = key

    def _next(self):
        self._k, sub = jax.random.split(self._k)
        return sub

    def normal(self, shape):
        return jax.random.normal(self._next(), shape, dtype=jnp.bfloat16)

    def randint(self, lo, hi, shape):
        return jax.random.randint(self._next(), shape, lo, hi, dtype=jnp.int32)

    def uniform(self, shape, lo=0.0, hi=1.0):
        return jax.random.uniform(self._next(), shape, jnp.bfloat16, lo, hi)

    def permutation(self, n):
        return jax.random.permutation(self._next(), n)
kernel_name = 'adaLN_cond__sliding_block__dense_activation_relu__prompt'

def setup_inputs():
    _rng = _Rng(jax.random.key(int.from_bytes(__import__("os").urandom(4), "little")))
    _w = lambda a: (lambda t: t.astype(jnp.bfloat16) if jnp.issubdtype(t.dtype, jnp.floating) else t)(jnp.asarray(a))

    def _A_setup():
        B, S, D = (1, 2048, 512)
        return {'x': _w((lambda *s: _rng.normal(s) * 0.05)(B, S, D)), 'wqkv': _w((lambda *s: _rng.normal(s) * 0.05)(D, 3 * D)), 'wo': _w((lambda *s: _rng.normal(s) * 0.05)(D, D))}
    _A_in = _A_setup()

    def _B_setup():
        B, S, D, Dff = (1, 2048, 512, 1792)
        return {'x': _w((lambda *s: _rng.normal(s) * 0.05)(B, S, D)), 'w1': _w((lambda *s: _rng.normal(s) * 0.05)(D, Dff)), 'w2': _w((lambda *s: _rng.normal(s) * 0.05)(Dff, D))}
    _B_in = _B_setup()
    return {'A_x': _A_in['x'], 'A_wqkv': _A_in['wqkv'], 'A_wo': _A_in['wo'], 'B_x': _B_in['x'], 'B_w1': _B_in['w1'], 'B_w2': _B_in['w2'], 'c': _w((lambda *s: _rng.normal(s) * 0.05)(1, 512) * 8.0), 'w_mod': _w((lambda *s: _rng.normal(s) * 0.05)(512, 6 * 512) * 512 ** (-0.5) * 8.0)}

def reference(A_x, A_wqkv, A_wo, B_x, B_w1, B_w2, c, w_mod):

    def _A_ref(x, wqkv, wo):
        B, S, D = x.shape
        H = 32
        Dh = D // H
        W = 256
        qkv = (lambda x, *d: x.transpose(*d))((x @ wqkv).reshape(B, S, 3, H, Dh), 2, 0, 3, 1, 4)
        q, k, v = (qkv[0], qkv[1], qkv[2])
        scores = jnp.einsum('bhqd,bhkd->bhqk', q, k) * Dh ** (-0.5)
        idx = jnp.arange(S)
        mask = (idx[:, None] - idx[None, :] >= 0) & (idx[:, None] - idx[None, :] < W)
        scores = jnp.where(mask[None, None], scores, -1000000000.0)
        p = _softmax(scores, axis=-1)
        o = jnp.einsum('bhqk,bhkd->bhqd', p, v)
        return (lambda x, *d: x.transpose(*d))(o, 0, 2, 1, 3).reshape(B, S, D) @ wo

    def _B_ref(x, w1, w2):
        h = jnp.einsum('bsd,df->bsf', x, w1)
        zero = jnp.zeros_like(h)
        h = jnp.maximum(h, zero)
        return jnp.einsum('bsf,fd->bsd', h, w2)
    x = A_x
    mod = (_silu(c) @ w_mod).reshape(c.shape[0], 6, 1, -1)
    sa, ca, ga, sb, cb, gb = (mod[:, 0].copy(), mod[:, 1].copy(), mod[:, 2].copy(), mod[:, 3].copy(), mod[:, 4].copy(), mod[:, 5].copy())
    h = _layernorm(x, axis=-1) * (1 + ca) + sa
    x = x + ga * _A_ref(h, A_wqkv, A_wo)
    h = _layernorm(x, axis=-1) * (1 + cb) + sb
    x = x + gb * _B_ref(h, B_w1, B_w2)
    return x
```

```python
import jax
import jax.numpy as jnp
import jax.experimental.pallas as pl
import jax.experimental.pallas.tpu as pltpu

F32 = jnp.float32
BF = jnp.bfloat16
U32 = jnp.uint32

S = 2048
D = 512
H = 32
DFF = 1792
T = 256
NBLK = S // T
EPS = 1e-5
QSCALE = 0.25 * 1.4426950408889634
NEG = -1e30
NT = (((1,), (1,)), ((), ()))

DA = 2
DB = 2
QK_CUTS = (0, 80, 160, 224, 288)

(SEM_C, SEM_WMA, SEM_WQ, SEM_WV, SEM_WK, SEM_WMB, SEM_WO, SEM_W1, SEM_W2) = range(9)
SEM_X0 = 9
NSEM = SEM_X0 + NBLK


def _u32(x):
    return x if x.dtype == U32 else pltpu.bitcast(x, U32)


def _pack_pairs(a, b):
    return _u32(pltpu.pack_elementwise([a, b], packed_dtype=BF))


def _layernorm(x):
    mu = jnp.mean(x, axis=-1, keepdims=True)
    xc = x - mu
    var = jnp.mean(xc * xc, axis=-1, keepdims=True)
    return xc * jax.lax.rsqrt(var + EPS)


def _kernel(x_hbm, wqkv_hbm, wo_hbm, w1_hbm, w2_hbm, c_hbm, wmod_hbm, out_ref,
            x_v, wq_v, wk_v, wv_v, wo_v, w1_v, w2_v, c_v, wmod_v,
            wqt_s, wvt_s, mod_s, hn_s, hp_s, k_s, k4_s, vt_s, qt_s, ot_s, l_s,
            x1_s, h2_s, sems):
    pid = pl.program_id(0)

    def cp(src, dst, slot):
        return pltpu.make_async_copy(src, dst, sems.at[slot])

    def x_copy(i):
        return cp(x_hbm.at[pl.ds(i * T, T), :], x_v.at[pl.ds(i * T, T), :], SEM_X0 + i)

    c_copy = cp(c_hbm, c_v, SEM_C)
    wma_copy = cp(wmod_hbm.at[:, pl.ds(0, 2 * D)], wmod_v.at[:, pl.ds(0, 2 * D)], SEM_WMA)
    wmb_copy = cp(wmod_hbm.at[:, pl.ds(2 * D, 4 * D)], wmod_v.at[:, pl.ds(2 * D, 4 * D)], SEM_WMB)
    wq_copy = cp(wqkv_hbm.at[:, pl.ds(0, D)], wq_v, SEM_WQ)
    wk_copy = cp(wqkv_hbm.at[:, pl.ds(D, D)], wk_v, SEM_WK)
    wv_copy = cp(wqkv_hbm.at[:, pl.ds(2 * D, D)], wv_v, SEM_WV)
    wo_copy = cp(wo_hbm, wo_v, SEM_WO)
    w1_copy = cp(w1_hbm, w1_v, SEM_W1)
    w2_copy = cp(w2_hbm, w2_v, SEM_W2)

    def mod_part(lo, hi):
        cf = c_v[...].astype(F32)
        sc = cf * (1.0 / (1.0 + jnp.exp(-cf)))
        sc = jnp.broadcast_to(sc, (16, D)).astype(BF)
        m = jnp.dot(sc, wmod_v[:, lo:hi], preferred_element_type=F32)
        mod_s[:, lo:hi] = m[0:8]

    def modrow(k):
        return mod_s[0:1, k * D:(k + 1) * D]

    def transpose_weight(w_v, wt_s):
        r = jax.lax.broadcasted_iota(jnp.int32, (128, 128), 0)
        f = jax.lax.broadcasted_iota(jnp.int32, (128, 128), 1)
        src = (r & ~15) + 2 * (r & 7) + ((r >> 3) & 1)
        pm = jnp.where(f == src, 1.0, 0.0).astype(BF)
        for ft in range(4):
            res = jax.lax.dot_general(pm, w_v[:, 128 * ft:128 * ft + 128], NT,
                                      preferred_element_type=F32)
            wt_s[128 * ft:128 * ft + 128, :] = res.astype(BF)

    def ln1(blk):
        r0 = pl.multiple_of(blk * T, T)
        xf = x_v[pl.ds(r0, T), :].astype(F32)
        h = _layernorm(xf) * (1.0 + modrow(1)) + modrow(0)
        hn_s[...] = h.astype(BF)
        hp = [_pack_pairs(h[16 * g:16 * g + 8], h[16 * g + 8:16 * g + 16]) for g in range(T // 16)]
        hp_s[...] = jnp.concatenate(hp, axis=0)

    def qkv(blk):
        hn = hn_s[...]
        hp = pltpu.bitcast(hp_s[...], BF)
        qt = jax.lax.dot_general(wqt_s[...], hn, NT, preferred_element_type=F32) * QSCALE
        for h in range(H):
            qt_s[8 * h:8 * h + 8, :] = _pack_pairs(qt[16 * h:16 * h + 8], qt[16 * h + 8:16 * h + 16])
        k = jnp.dot(hn, wk_v[...], preferred_element_type=F32)
        r0 = pl.multiple_of(blk * (T // 2) + 64, 64)
        k_s[pl.ds(r0, T // 2), :] = _u32(k.astype(BF))
        vt = jax.lax.dot_general(wvt_s[...], hp, NT, preferred_element_type=F32)
        for b in range(T // 128):
            pk = [_pack_pairs(vt[16 * h:16 * h + 8, 128 * b:128 * b + 128],
                              vt[16 * h + 8:16 * h + 16, 128 * b:128 * b + 128]) for h in range(H)]
            vt_s[blk * (T // 128) + b] = jnp.concatenate(pk, axis=0)

    def k4_build(blk):
        lane = jax.lax.broadcasted_iota(jnp.int32, (8, 128), 1)
        lt = [lane < 32 * s for s in range(4)]
        src0 = blk * (T // 2) + 64 - 48
        dst0 = blk * (T // 2)
        nu = T // 16
        for g in range(4):
            rolled = {}

            def kv(w, d, g=g, rolled=rolled):
                if (w, d) not in rolled:
                    if d == 0:
                        rolled[(w, 0)] = k_s[pl.ds(pl.multiple_of(src0 + 8 * w, 8), 8),
                                             128 * g:128 * g + 128]
                    else:
                        rolled[(w, d)] = pltpu.roll(kv(w, 0), 32 * d, 1)
                return rolled[(w, d)]

            for u in range(nu):
                for pp in range(4):
                    c = [kv(u + 2 * s, (s - pp) % 4) for s in range(4)]
                    o = jnp.where(lt[2], jnp.where(lt[1], c[0], c[1]), jnp.where(lt[3], c[2], c[3]))
                    k4_s[4 * g + pp, pl.ds(pl.multiple_of(dst0 + 8 * u, 8), 8), :] = o

    def attention(blk, first):
        lane8 = jax.lax.broadcasted_iota(jnp.int32, (8, 128), 1)
        srow = jax.lax.broadcasted_iota(jnp.int32, (8, 128), 0)
        i8 = lane8 & 31
        first_m = [8 * v + srow > i8 for v in range(4)]
        last_m = [8 * v + srow <= i8 for v in range(4)]
        blkid = lane8 >> 5
        blkm = [blkid == s for s in range(4)]
        blkge = [blkid >= s for s in range(4)]
        odd = (blkid & 1) == 1
        hi2 = blkid >= 2
        zero8 = jnp.zeros((8, 128), U32)
        neg8 = jnp.full((8, 128), NEG, F32)

        def st_a(b, h):
            nneg = max(0, 256 - 128 * b) if first else 0
            tmin = max(0, nneg - 96)
            p, hh = h // 2, h % 2
            qv = qt_s[8 * h:8 * h + 8, 128 * b:128 * b + 128]
            parts = [zero8] * 8
            for s in range(4):
                parts[2 * s + hh] = jnp.where(blkm[s], qv, zero8)
            w = pltpu.bitcast(jnp.concatenate(parts, axis=0), BF)
            row0 = blk * (T // 2) + 64 * b - 80
            if tmin == 0:
                cuts = QK_CUTS
            elif tmin == 32:
                cuts = (32, 96, 160, 224, 288)
            else:
                cuts = (160, 192, 224, 256, 288)
            sv = {}
            for a_, b_ in zip(cuts[:-1], cuts[1:]):
                kc = k4_s[p, pl.ds(pl.multiple_of(row0 + a_ // 2, 8), (b_ - a_) // 2), :]
                sc = jnp.dot(pltpu.bitcast(kc, BF), w, preferred_element_type=F32)
                for v in range((b_ - a_) // 8):
                    sv[a_ // 8 + v] = sc[8 * v:8 * v + 8]
            for v in sorted(sv):
                if v < 4:
                    sv[v] = jnp.where(first_m[v], sv[v], neg8)
                elif v >= 32:
                    sv[v] = jnp.where(last_m[v - 32], sv[v], neg8)
                if 8 * v < nneg:
                    smin = -((8 * v - nneg) // 32)
                    sv[v] = jnp.where(blkge[smin], sv[v], neg8)
            vs = sorted(sv)
            m0, m1 = sv[vs[0]], sv[vs[1]]
            for v in vs[2::2]:
                m0 = jnp.maximum(m0, sv[v])
                m1 = jnp.maximum(m1, sv[v + 1])
            m = jnp.max(jnp.maximum(m0, m1), axis=0, keepdims=True)
            return jnp.broadcast_to(m, (8, 128)), sv

        def st_b(b, h, st):
            m, sv = st
            c0 = max(0, 2 - b) if first else 0
            pf, bb, outv = {}, {}, []

            def sel(mk, a, c):
                if a is None and c is None:
                    return None
                return jnp.where(mk, zero8 if a is None else a, zero8 if c is None else c)

            l0 = l1 = None
            for v in range(24):
                if v < 18 and 2 * v in sv:
                    a = jnp.exp2(sv[2 * v] - m)
                    c = jnp.exp2(sv[2 * v + 1] - m)
                    l0 = a if l0 is None else l0 + a
                    l1 = c if l1 is None else l1 + c
                    pf[v] = _pack_pairs(a, c)
                if v < 20:
                    bb[v] = sel(odd, pf.get(v - 2), pf.get(v))
                if v >= 8 * c0:
                    o = sel(hi2, bb.get(v - 4), bb.get(v))
                    outv.append(zero8 if o is None else o)
            l_s[h:h + 1, 128 * b:128 * b + 128] = jnp.sum(l0 + l1, axis=0, keepdims=True)
            return outv

        def st_c(b, h, outv):
            c0 = max(0, 2 - b) if first else 0
            pfull = pltpu.bitcast(jnp.concatenate(outv, axis=0), BF)
            tile0 = blk * (T // 128) + b - 2
            vt = jnp.concatenate([vt_s[tile0 + c, 8 * h:8 * h + 8, :] for c in range(c0, 3)], axis=1)
            o = jnp.dot(pltpu.bitcast(vt, BF), pfull, preferred_element_type=F32)
            ot_s[16 * h:16 * h + 16, 128 * b:128 * b + 128] = o

        items = [(b, h) for b in range(T // 128) for h in range(H)]
        n = len(items)
        sa, sb = {}, {}
        for t in range(n + DA + DB):
            if t < n:
                sa[t] = st_a(*items[t])
            u = t - DA
            if 0 <= u < n:
                sb[u] = st_b(*items[u], sa.pop(u))
            w = t - DA - DB
            if 0 <= w < n:
                st_c(*items[w], sb.pop(w))

    def attn_out(blk):
        rl = 1.0 / l_s[...]
        parts = [ot_s[16 * h:16 * h + 16, :] * rl[h:h + 1, :] for h in range(H)]
        o = jnp.concatenate(parts, axis=0).T.astype(BF)
        z = jnp.dot(o, wo_v[...], preferred_element_type=F32)
        r0 = pl.multiple_of(blk * T, T)
        x1 = x_v[pl.ds(r0, T), :].astype(F32) + modrow(2) * z
        x1_s[...] = x1
        h2 = _layernorm(x1) * (1.0 + modrow(4)) + modrow(3)
        h2_s[...] = h2.astype(BF)

    def ffn():
        a = jnp.dot(h2_s[...], w1_v[...], preferred_element_type=F32)
        a = jnp.maximum(a, 0.0).astype(BF)
        y = jnp.dot(a, w2_v[...], preferred_element_type=F32)
        out_ref[...] = (x1_s[...] + modrow(5) * y).astype(out_ref.dtype)

    @pl.when(pid == 0)
    def _():
        x_copy(0).start()
        c_copy.start()
        wma_copy.start()
        wq_copy.start()
        wv_copy.start()
        wk_copy.start()
        k_s[0:64, :] = jnp.zeros((64, D), U32)
        c_copy.wait()
        wma_copy.wait()
        mod_part(0, 2 * D)
        x_copy(0).wait()
        ln1(0)
        wq_copy.wait()
        transpose_weight(wq_v, wqt_s)
        wv_copy.wait()
        transpose_weight(wv_v, wvt_s)
        wk_copy.wait()
        x_copy(1).start()
        wmb_copy.start()
        wo_copy.start()
        w1_copy.start()
        w2_copy.start()
        for i in range(2, NBLK):
            x_copy(i).start()
        qkv(0)
        k4_build(0)
        attention(0, True)
        wmb_copy.wait()
        mod_part(2 * D, 6 * D)
        wo_copy.wait()
        attn_out(0)
        w1_copy.wait()
        w2_copy.wait()
        ffn()
        for i in range(1, NBLK):
            x_copy(i).wait()

    @pl.when(pid > 0)
    def _():
        ln1(pid)
        qkv(pid)
        k4_build(pid)
        attention(pid, False)
        attn_out(pid)
        ffn()


@jax.jit
def pallas_adaLN_cond__sliding_block__dense_activation_relu__prompt_kernel(
    A_x: jax.Array,
    A_wqkv: jax.Array,
    A_wo: jax.Array,
    B_x: jax.Array,
    B_w1: jax.Array,
    B_w2: jax.Array,
    c: jax.Array,
    w_mod: jax.Array,
):
    del B_x
    x = A_x.reshape(S, D)
    any_spec = pl.BlockSpec(memory_space=pl.ANY)
    scratch = [
        pltpu.VMEM((S, D), BF),
        pltpu.VMEM((D, D), BF),
        pltpu.VMEM((D, D), BF),
        pltpu.VMEM((D, D), BF),
        pltpu.VMEM((D, D), BF),
        pltpu.VMEM((D, DFF), BF),
        pltpu.VMEM((DFF, D), BF),
        pltpu.VMEM((1, D), BF),
        pltpu.VMEM((D, 6 * D), BF),
        pltpu.VMEM((D, D), BF),
        pltpu.VMEM((D, D), BF),
        pltpu.VMEM((8, 6 * D), F32),
        pltpu.VMEM((T, D), BF),
        pltpu.VMEM((T // 2, D), U32),
        pltpu.VMEM((S // 2 + 64, D), U32),
        pltpu.VMEM((16, S // 2, 128), U32),
        pltpu.VMEM((S // 128, D // 2, 128), U32),
        pltpu.VMEM((D // 2, T), U32),
        pltpu.VMEM((D, T), F32),
        pltpu.VMEM((H, T), F32),
        pltpu.VMEM((T, D), F32),
        pltpu.VMEM((T, D), BF),
        pltpu.SemaphoreType.DMA((NSEM,)),
    ]
    out = pl.pallas_call(
        _kernel,
        grid=(NBLK,),
        in_specs=[any_spec] * 7,
        out_specs=pl.BlockSpec((T, D), lambda i: (i, 0)),
        out_shape=jax.ShapeDtypeStruct((S, D), BF),
        scratch_shapes=scratch,
        compiler_params=pltpu.CompilerParams(
            dimension_semantics=("arbitrary",),
            vmem_limit_bytes=100 * 1024 * 1024),
    )(x, A_wqkv, A_wo, B_w1, B_w2, c, w_mod)
    return out.reshape(1, S, D)
```

```python
import jax
import jax.numpy as jnp
import jax.experimental.pallas as pl
import jax.experimental.pallas.tpu as pltpu

F32 = jnp.float32
BF = jnp.bfloat16
U32 = jnp.uint32

S = 2048
D = 512
H = 32
DFF = 1792
T = 256
NBLK = S // T
EPS = 1e-5
QSCALE = 0.25 * 1.4426950408889634
NEG = -1e30
NT = (((1,), (1,)), ((), ()))

W2WAIT = 1
LNR = 16
LN1POS = 0
FILL_N = 1
FILL_T0 = 64
FILL_DT = 16
TAIL0 = 0
DA = 2
DB = 2
QK_CUTS = (0, 80, 160, 224, 288)

(SEM_C, SEM_WMA, SEM_WQ, SEM_WV, SEM_WK, SEM_WMB, SEM_WO, SEM_W1, SEM_W2, SEM_WMC) = range(10)
SEM_X0 = 10
NSEM = SEM_X0 + NBLK


def _u32(x):
    return x if x.dtype == U32 else pltpu.bitcast(x, U32)


def _pack_pairs(a, b):
    return _u32(pltpu.pack_elementwise([a, b], packed_dtype=BF))


def _layernorm(x):
    mu = jnp.mean(x, axis=-1, keepdims=True)
    xc = x - mu
    var = jnp.mean(xc * xc, axis=-1, keepdims=True)
    return xc * jax.lax.rsqrt(var + EPS)


def _kernel(x_hbm, wqkv_hbm, wo_hbm, w1_hbm, w2_hbm, c_hbm, wmod_hbm, out_ref,
            x_v, wq_v, wk_v, wv_v, wo_v, w1_v, w2_v, c_v, wmod_v,
            wqt_s, wvt_s, mod_s, hn_s, hp_s, k_s, k4_s, vt_s, qt_s, ot_s, l_s,
            x1_s, h2_s, x1c_s, a_s, sems):
    pid = pl.program_id(0)

    def cp(src, dst, slot):
        return pltpu.make_async_copy(src, dst, sems.at[slot])

    def x_copy(i):
        return cp(x_hbm.at[pl.ds(i * T, T), :], x_v.at[pl.ds(i * T, T), :], SEM_X0 + i)

    c_copy = cp(c_hbm, c_v, SEM_C)
    wma_copy = cp(wmod_hbm.at[:, pl.ds(0, 2 * D)], wmod_v.at[:, pl.ds(0, 2 * D)], SEM_WMA)
    wmb_copy = cp(wmod_hbm.at[:, pl.ds(2 * D, 4 * D)], wmod_v.at[:, pl.ds(2 * D, 4 * D)], SEM_WMB)
    wq_copy = cp(wqkv_hbm.at[:, pl.ds(0, D)], wq_v, SEM_WQ)
    wk_copy = cp(wqkv_hbm.at[:, pl.ds(D, D)], wk_v, SEM_WK)
    wv_copy = cp(wqkv_hbm.at[:, pl.ds(2 * D, D)], wv_v, SEM_WV)
    wo_copy = cp(wo_hbm, wo_v, SEM_WO)
    w1_copy = cp(w1_hbm, w1_v, SEM_W1)
    w2_copy = cp(w2_hbm, w2_v, SEM_W2)

    def mod_part(lo, hi):
        cf = c_v[...].astype(F32)
        sc = cf * (1.0 / (1.0 + jnp.exp(-cf)))
        sc = jnp.broadcast_to(sc, (16, D)).astype(BF)
        m = jnp.dot(sc, wmod_v[:, lo:hi], preferred_element_type=F32)
        mod_s[:, lo:hi] = m[0:8]

    def modrow(k):
        return mod_s[0:1, k * D:(k + 1) * D]

    def transpose_weight(w_v, wt_s):
        r = jax.lax.broadcasted_iota(jnp.int32, (128, 128), 0)
        f = jax.lax.broadcasted_iota(jnp.int32, (128, 128), 1)
        src = (r & ~15) + 2 * (r & 7) + ((r >> 3) & 1)
        pm = jnp.where(f == src, 1.0, 0.0).astype(BF)
        for ft in range(4):
            res = jax.lax.dot_general(pm, w_v[:, 128 * ft:128 * ft + 128], NT,
                                      preferred_element_type=F32)
            wt_s[128 * ft:128 * ft + 128, :] = res.astype(BF)

    def ln1(blk):
        r0 = pl.multiple_of(blk * T, T)
        g1 = 1.0 + modrow(1)
        sh = modrow(0)
        for r in range(0, T, LNR):
            xf = x_v[pl.ds(r0 + r, LNR), :].astype(F32)
            h = _layernorm(xf) * g1 + sh
            hn_s[r:r + LNR, :] = h.astype(BF)
            for g in range(LNR // 16):
                hp_s[r // 2 + 8 * g:r // 2 + 8 * g + 8, :] = _pack_pairs(
                    h[16 * g:16 * g + 8], h[16 * g + 8:16 * g + 16])

    def q_part():
        qt = jax.lax.dot_general(wqt_s[...], hn_s[...], NT, preferred_element_type=F32) * QSCALE
        for h in range(H):
            qt_s[8 * h:8 * h + 8, :] = _pack_pairs(qt[16 * h:16 * h + 8], qt[16 * h + 8:16 * h + 16])

    def k_part(blk):
        k = jnp.dot(hn_s[...], wk_v[...], preferred_element_type=F32)
        r0 = pl.multiple_of(blk * (T // 2) + 64, 64)
        k_s[pl.ds(r0, T // 2), :] = _u32(k.astype(BF))

    def v_part(blk):
        hp = pltpu.bitcast(hp_s[...], BF)
        vt = jax.lax.dot_general(wvt_s[...], hp, NT, preferred_element_type=F32)
        for b in range(T // 128):
            pk = [_pack_pairs(vt[16 * h:16 * h + 8, 128 * b:128 * b + 128],
                              vt[16 * h + 8:16 * h + 16, 128 * b:128 * b + 128]) for h in range(H)]
            vt_s[blk * (T // 128) + b] = jnp.concatenate(pk, axis=0)

    def k4_build(blk):
        lane = jax.lax.broadcasted_iota(jnp.int32, (8, 128), 1)
        lt = [lane < 32 * s for s in range(4)]
        src0 = blk * (T // 2) + 64 - 48
        dst0 = blk * (T // 2)
        nu = T // 16
        for g in range(4):
            rolled = {}

            def kv(w, d, g=g, rolled=rolled):
                if (w, d) not in rolled:
                    if d == 0:
                        rolled[(w, 0)] = k_s[pl.ds(pl.multiple_of(src0 + 8 * w, 8), 8),
                                             128 * g:128 * g + 128]
                    else:
                        rolled[(w, d)] = pltpu.roll(kv(w, 0), 32 * d, 1)
                return rolled[(w, d)]

            for u in range(nu):
                for pp in range(4):
                    c = [kv(u + 2 * s, (s - pp) % 4) for s in range(4)]
                    o = jnp.where(lt[2], jnp.where(lt[1], c[0], c[1]), jnp.where(lt[3], c[2], c[3]))
                    k4_s[4 * g + pp, pl.ds(pl.multiple_of(dst0 + 8 * u, 8), 8), :] = o

    def attention(blk, first, fillers=None):
        lane8 = jax.lax.broadcasted_iota(jnp.int32, (8, 128), 1)
        srow = jax.lax.broadcasted_iota(jnp.int32, (8, 128), 0)
        i8 = lane8 & 31
        first_m = [8 * v + srow > i8 for v in range(4)]
        last_m = [8 * v + srow <= i8 for v in range(4)]
        blkid = lane8 >> 5
        blkm = [blkid == s for s in range(4)]
        blkge = [blkid >= s for s in range(4)]
        odd = (blkid & 1) == 1
        hi2 = blkid >= 2
        zero8 = jnp.zeros((8, 128), U32)
        neg8 = jnp.full((8, 128), NEG, F32)

        def st_a(b, h):
            nneg = max(0, 256 - 128 * b) if first else 0
            tmin = max(0, nneg - 96)
            p, hh = h // 2, h % 2
            qv = qt_s[8 * h:8 * h + 8, 128 * b:128 * b + 128]
            parts = [zero8] * 8
            for s in range(4):
                parts[2 * s + hh] = jnp.where(blkm[s], qv, zero8)
            w = pltpu.bitcast(jnp.concatenate(parts, axis=0), BF)
            row0 = blk * (T // 2) + 64 * b - 80
            if tmin == 0:
                cuts = QK_CUTS
            elif tmin == 32:
                cuts = (32, 96, 160, 224, 288)
            else:
                cuts = (160, 192, 224, 256, 288)
            sv = {}
            for a_, b_ in zip(cuts[:-1], cuts[1:]):
                kc = k4_s[p, pl.ds(pl.multiple_of(row0 + a_ // 2, 8), (b_ - a_) // 2), :]
                sc = jnp.dot(pltpu.bitcast(kc, BF), w, preferred_element_type=F32)
                for v in range((b_ - a_) // 8):
                    sv[a_ // 8 + v] = sc[8 * v:8 * v + 8]
            for v in sorted(sv):
                if v < 4:
                    sv[v] = jnp.where(first_m[v], sv[v], neg8)
                elif v >= 32:
                    sv[v] = jnp.where(last_m[v - 32], sv[v], neg8)
                if 8 * v < nneg:
                    smin = -((8 * v - nneg) // 32)
                    sv[v] = jnp.where(blkge[smin], sv[v], neg8)
            vs = sorted(sv)
            m0, m1 = sv[vs[0]], sv[vs[1]]
            for v in vs[2::2]:
                m0 = jnp.maximum(m0, sv[v])
                m1 = jnp.maximum(m1, sv[v + 1])
            m = jnp.max(jnp.maximum(m0, m1), axis=0, keepdims=True)
            return jnp.broadcast_to(m, (8, 128)), sv

        def st_b(b, h, st):
            m, sv = st
            c0 = max(0, 2 - b) if first else 0
            pf, bb, outv = {}, {}, []

            def sel(mk, a, c):
                if a is None and c is None:
                    return None
                return jnp.where(mk, zero8 if a is None else a, zero8 if c is None else c)

            l0 = l1 = None
            for v in range(24):
                if v < 18 and 2 * v in sv:
                    a = jnp.exp2(sv[2 * v] - m)
                    c = jnp.exp2(sv[2 * v + 1] - m)
                    l0 = a if l0 is None else l0 + a
                    l1 = c if l1 is None else l1 + c
                    pf[v] = _pack_pairs(a, c)
                if v < 20:
                    bb[v] = sel(odd, pf.get(v - 2), pf.get(v))
                if v >= 8 * c0:
                    o = sel(hi2, bb.get(v - 4), bb.get(v))
                    outv.append(zero8 if o is None else o)
            l_s[h:h + 1, 128 * b:128 * b + 128] = jnp.sum(l0 + l1, axis=0, keepdims=True)
            return outv

        def st_c(b, h, outv):
            c0 = max(0, 2 - b) if first else 0
            pfull = pltpu.bitcast(jnp.concatenate(outv, axis=0), BF)
            tile0 = blk * (T // 128) + b - 2
            vt = jnp.concatenate([vt_s[tile0 + c, 8 * h:8 * h + 8, :] for c in range(c0, 3)], axis=1)
            o = jnp.dot(pltpu.bitcast(vt, BF), pfull, preferred_element_type=F32)
            ot_s[16 * h:16 * h + 16, 128 * b:128 * b + 128] = o

        items = [(b, h) for b in range(T // 128) for h in range(H)]
        n = len(items)
        sa, sb = {}, {}
        for t in range(n + DA + DB):
            if t < n:
                sa[t] = st_a(*items[t])
            if fillers is not None and t in fillers:
                for f in fillers[t]:
                    f()
            u = t - DA
            if 0 <= u < n:
                sb[u] = st_b(*items[u], sa.pop(u))
            w = t - DA - DB
            if 0 <= w < n:
                st_c(*items[w], sb.pop(w))

    def attn_proj(lo, hi):
        rl = 1.0 / l_s[:, lo:hi]
        parts = [ot_s[16 * h:16 * h + 16, lo:hi] * rl[h:h + 1, :] for h in range(H)]
        o = jnp.concatenate(parts, axis=0).T.astype(BF)
        return jnp.dot(o, wo_v[...], preferred_element_type=F32)

    def ln2(blk, z, lo, hi):
        r0 = pl.multiple_of(blk * T + lo, 128)
        g2 = 1.0 + modrow(4)
        sh = modrow(3)
        ga = modrow(2)
        for r in range(0, hi - lo, LNR):
            x1 = x_v[pl.ds(r0 + r, LNR), :].astype(F32) + ga * z[r:r + LNR]
            x1_s[lo + r:lo + r + LNR, :] = x1
            h2 = _layernorm(x1) * g2 + sh
            h2_s[lo + r:lo + r + LNR, :] = h2.astype(BF)

    def ffn_up():
        a = jnp.dot(h2_s[...], w1_v[...], preferred_element_type=F32)
        a_s[...] = jnp.maximum(a, 0.0).astype(BF)

    def ffn_down(res_ref, rlo, lo, hi, c0=0, c1=D):
        y = jnp.dot(a_s[lo:hi, :], w2_v[:, c0:c1], preferred_element_type=F32)
        gb = mod_s[0:1, 5 * D + c0:5 * D + c1]
        out_ref[lo:hi, c0:c1] = (res_ref[rlo:rlo + hi - lo, c0:c1] + gb * y).astype(out_ref.dtype)

    HT = T // 2

    @pl.when(pid == 0)
    @jax.named_scope("first")
    def _():
        for cpy in (c_copy, x_copy(0), wma_copy, wk_copy, wq_copy, wv_copy, wo_copy,
                    wmb_copy, x_copy(1), w1_copy, x_copy(2), w2_copy):
            cpy.start()
        for i in range(3, NBLK):
            x_copy(i).start()
        k_s[0:64, :] = jnp.zeros((64, D), U32)
        c_copy.wait()
        x_copy(0).wait()
        wma_copy.wait()
        mod_part(0, 2 * D)
        ln1(0)
        wk_copy.wait()
        k_part(0)
        wq_copy.wait()
        transpose_weight(wq_v, wqt_s)
        q_part()
        k4_build(0)
        wv_copy.wait()
        transpose_weight(wv_v, wvt_s)
        v_part(0)
        attention(0, True)
        wo_copy.wait()
        wmb_copy.wait()
        x_copy(1).wait()
        mod_part(2 * D, 6 * D)
        ln2(0, attn_proj(0, T), 0, T)
        ln1(1)
        w1_copy.wait()
        ffn_up()

    @pl.when((pid >= 1) & (pid < NBLK - 1))
    def _():
        x_copy(pid + 1).wait()

    pl.when(pid == 1)(w2_copy.wait)

    @pl.when((pid >= 1) & (pid < NBLK))
    @jax.named_scope("mid")
    def _():
        nxt = jnp.minimum(pid + 1, NBLK - 1)
        q_part()
        k_part(pid)
        v_part(pid)
        k4_build(pid)
        if LN1POS == 0:
            ln1(nxt)
        fill = {}
        ng = (T // 128) * H
        for j in range(FILL_N):
            cw = D // FILL_N
            t = FILL_T0 + j * FILL_DT
            fill.setdefault(t, []).append(
                lambda j=j, cw=cw: ffn_down(x1_s, 0, 0, HT, j * cw, (j + 1) * cw))
        if TAIL0:
            fill.setdefault(H + DA + DB, []).append(lambda: ln2(pid, attn_proj(0, HT), 0, HT))
        attention(pid, False, fill)
        if TAIL0:
            x1c_s[...] = x1_s[HT:T, :]
            ffn_down(x1c_s, 0, HT, T)
            ln2(pid, attn_proj(HT, T), HT, T)
        else:
            z = attn_proj(0, T)
            x1c_s[...] = x1_s[HT:T, :]
            ffn_down(x1c_s, 0, HT, T)
            ln2(pid, z, 0, T)
        if LN1POS == 1:
            ln1(nxt)
        ffn_up()
        if LN1POS == 2:
            ln1(nxt)

    @pl.when(pid == NBLK)
    @jax.named_scope("last")
    def _():
        ffn_down(x1_s, 0, 0, T)


@jax.jit
def pallas_adaLN_cond__sliding_block__dense_activation_relu__prompt_kernel(
    A_x: jax.Array,
    A_wqkv: jax.Array,
    A_wo: jax.Array,
    B_x: jax.Array,
    B_w1: jax.Array,
    B_w2: jax.Array,
    c: jax.Array,
    w_mod: jax.Array,
):
    del B_x
    x = A_x.reshape(S, D)
    any_spec = pl.BlockSpec(memory_space=pl.ANY)
    scratch = [
        pltpu.VMEM((S, D), BF),
        pltpu.VMEM((D, D), BF),
        pltpu.VMEM((D, D), BF),
        pltpu.VMEM((D, D), BF),
        pltpu.VMEM((D, D), BF),
        pltpu.VMEM((D, DFF), BF),
        pltpu.VMEM((DFF, D), BF),
        pltpu.VMEM((1, D), BF),
        pltpu.VMEM((D, 6 * D), BF),
        pltpu.VMEM((D, D), BF),
        pltpu.VMEM((D, D), BF),
        pltpu.VMEM((8, 6 * D), F32),
        pltpu.VMEM((T, D), BF),
        pltpu.VMEM((T // 2, D), U32),
        pltpu.VMEM((S // 2 + 64, D), U32),
        pltpu.VMEM((16, S // 2, 128), U32),
        pltpu.VMEM((S // 128, D // 2, 128), U32),
        pltpu.VMEM((D // 2, T), U32),
        pltpu.VMEM((D, T), F32),
        pltpu.VMEM((H, T), F32),
        pltpu.VMEM((T, D), F32),
        pltpu.VMEM((T, D), BF),
        pltpu.VMEM((T // 2, D), F32),
        pltpu.VMEM((T, DFF), BF),
        pltpu.SemaphoreType.DMA((NSEM,)),
    ]
    out = pl.pallas_call(
        _kernel,
        grid=(NBLK + 1,),
        in_specs=[any_spec] * 7,
        out_specs=pl.BlockSpec((T, D), lambda i: (jnp.maximum(i - 1, 0), 0)),
        out_shape=jax.ShapeDtypeStruct((S, D), BF),
        scratch_shapes=scratch,
        compiler_params=pltpu.CompilerParams(
            dimension_semantics=("arbitrary",),
            vmem_limit_bytes=100 * 1024 * 1024),
    )(x, A_wqkv, A_wo, B_w1, B_w2, c, w_mod)
    return out.reshape(1, S, D)
```

```python
import jax
import jax.numpy as jnp
import jax.experimental.pallas as pl
import jax.experimental.pallas.tpu as pltpu

F32 = jnp.float32
BF = jnp.bfloat16
U32 = jnp.uint32

S = 2048
D = 512
H = 32
DFF = 1792
T = 256
NBLK = S // T
EPS = 1e-5
QSCALE = 0.25 * 1.4426950408889634
NEG = -1e30
NT = (((1,), (1,)), ((), ()))

W2WAIT = 1
LNR = 16
LN1POS = 1
FRONTPOS = 0
FILL_N = 1
FILL_T0 = 64
FILL_DT = 16
TAIL0 = 0
PRELN = 1
K8POS = 0
MODC = 1
QPOS = 1
MODB = 0
CUTS0 = (144,208,272)
CUTS1 = (16,112,192,272)
W1POS = 1
DA0 = 4
DB0 = 3
DA = 2
DB = 2
QK_CUTS = (0,64,128,192,272)

(SEM_C, SEM_WMA, SEM_WQ, SEM_WV, SEM_WK, SEM_WMB, SEM_WO, SEM_W1, SEM_W2, SEM_WMC) = range(10)
SEM_X0 = 10
NSEM = SEM_X0 + NBLK


def _u32(x):
    return x if x.dtype == U32 else pltpu.bitcast(x, U32)


def _pack_pairs(a, b):
    return _u32(pltpu.pack_elementwise([a, b], packed_dtype=BF))


def _layernorm(x):
    mu = jnp.mean(x, axis=-1, keepdims=True)
    xc = x - mu
    var = jnp.mean(xc * xc, axis=-1, keepdims=True)
    return xc * jax.lax.rsqrt(var + EPS)


def _kernel(x_hbm, wqkv_hbm, wo_hbm, w1_hbm, w2_hbm, c_hbm, wmod_hbm, out_ref,
            x_v, wq_v, wk_v, wv_v, wo_v, w1_v, w2_v, c_v, wmod_v,
            wqt_s, wvt_s, mod_s, hn_s, hp_s, hn0_s, hp0_s, k_s, k4_s, vt_s, qt_s, ot_s, l_s,
            x1_s, h2_s, x1c_s, a_s, sems):
    pid = pl.program_id(0)

    def cp(src, dst, slot):
        return pltpu.make_async_copy(src, dst, sems.at[slot])

    def x_copy(i):
        return cp(x_hbm.at[pl.ds(i * T, T), :], x_v.at[pl.ds(i * T, T), :], SEM_X0 + i)

    c_copy = cp(c_hbm, c_v, SEM_C)
    wma_copy = cp(wmod_hbm.at[:, pl.ds(0, 2 * D)], wmod_v.at[:, pl.ds(0, 2 * D)], SEM_WMA)
    wmb_copy = cp(wmod_hbm.at[:, pl.ds(2 * D, 3 * D)], wmod_v.at[:, pl.ds(2 * D, 3 * D)], SEM_WMB)
    wmc_copy = cp(wmod_hbm.at[:, pl.ds(5 * D, D)], wmod_v.at[:, pl.ds(5 * D, D)], SEM_WMC)
    wq_copy = cp(wqkv_hbm.at[:, pl.ds(0, D)], wq_v, SEM_WQ)
    wk_copy = cp(wqkv_hbm.at[:, pl.ds(D, D)], wk_v, SEM_WK)
    wv_copy = cp(wqkv_hbm.at[:, pl.ds(2 * D, D)], wv_v, SEM_WV)
    wo_copy = cp(wo_hbm, wo_v, SEM_WO)
    w1_copy = cp(w1_hbm, w1_v, SEM_W1)
    w2_copy = cp(w2_hbm, w2_v, SEM_W2)

    def mod_part(lo, hi):
        cf = c_v[...].astype(F32)
        sc = cf * (1.0 / (1.0 + jnp.exp(-cf)))
        sc = jnp.broadcast_to(sc, (16, D)).astype(BF)
        m = jnp.dot(sc, wmod_v[:, lo:hi], preferred_element_type=F32)
        mod_s[:, lo:hi] = m[0:8]

    def modrow(k):
        return mod_s[0:1, k * D:(k + 1) * D]

    def transpose_weight(w_v, wt_s):
        r = jax.lax.broadcasted_iota(jnp.int32, (128, 128), 0)
        f = jax.lax.broadcasted_iota(jnp.int32, (128, 128), 1)
        src = (r & ~15) + 2 * (r & 7) + ((r >> 3) & 1)
        pm = jnp.where(f == src, 1.0, 0.0).astype(BF)
        for ft in range(4):
            res = jax.lax.dot_general(pm, w_v[:, 128 * ft:128 * ft + 128], NT,
                                      preferred_element_type=F32)
            wt_s[128 * ft:128 * ft + 128, :] = res.astype(BF)

    def ln1_pre(blk):
        for r in range(0, T, LNR):
            x1_s[r:r + LNR, :] = _layernorm(x_v[blk * T + r:blk * T + r + LNR, :].astype(F32))

    def ln1(blk, hn_s=hn_s, hp_s=hp_s, pre=False):
        r0 = pl.multiple_of(blk * T, T)
        g1 = 1.0 + modrow(1)
        sh = modrow(0)
        for r in range(0, T, LNR):
            if pre:
                xn = x1_s[r:r + LNR, :]
            else:
                xn = _layernorm(x_v[pl.ds(r0 + r, LNR), :].astype(F32))
            h = xn * g1 + sh
            hn_s[r:r + LNR, :] = h.astype(BF)
            for g in range(LNR // 16):
                hp_s[r // 2 + 8 * g:r // 2 + 8 * g + 8, :] = _pack_pairs(
                    h[16 * g:16 * g + 8], h[16 * g + 8:16 * g + 16])

    def q_part(hn_s=hn_s):
        qt = jax.lax.dot_general(wqt_s[...], hn_s[...], NT, preferred_element_type=F32) * QSCALE
        for h in range(H):
            qt_s[8 * h:8 * h + 8, :] = _pack_pairs(qt[16 * h:16 * h + 8], qt[16 * h + 8:16 * h + 16])

    def k_part(blk, hn_s=hn_s):
        k = jnp.dot(hn_s[...], wk_v[...], preferred_element_type=F32)
        r0 = pl.multiple_of(blk * (T // 2) + 64, 64)
        k_s[pl.ds(r0, T // 2), :] = _u32(k.astype(BF))

    def v_part(blk, hp_s=hp_s):
        hp = pltpu.bitcast(hp_s[...], BF)
        vt = jax.lax.dot_general(wvt_s[...], hp, NT, preferred_element_type=F32)
        for b in range(T // 128):
            pk = [_pack_pairs(vt[16 * h:16 * h + 8, 128 * b:128 * b + 128],
                              vt[16 * h + 8:16 * h + 16, 128 * b:128 * b + 128]) for h in range(H)]
            vt_s[blk * (T // 128) + b] = jnp.concatenate(pk, axis=0)

    def k4_build(blk):
        lane = jax.lax.broadcasted_iota(jnp.int32, (8, 128), 1)
        bit = [((lane >> (4 + k)) & 1) == 1 for k in range(3)]
        src0 = blk * (T // 2) + 8
        dst0 = blk * (T // 2)
        for g in range(4):
            xs = {}

            def x(w, g=g, xs=xs):
                if w not in xs:
                    xs[w] = k_s[pl.ds(pl.multiple_of(src0 + 8 * w, 8), 8), 128 * g:128 * g + 128]
                return xs[w]

            for u in range(T // 16):
                f = [x(u)] + [pltpu.roll(x(u + d), 16 * d, 1) for d in range(1, 8)]
                for k in range(3):
                    f = [jnp.where(bit[k], f[(m + (1 << k)) % 8], f[m]) for m in range(8)]
                for hh in range(8):
                    k4_s[8 * g + hh, pl.ds(pl.multiple_of(dst0 + 8 * u, 8), 8), :] = f[(-hh) % 8]

    def attention(blk, first, fillers=None):
        lane8 = jax.lax.broadcasted_iota(jnp.int32, (8, 128), 1)
        srow = jax.lax.broadcasted_iota(jnp.int32, (8, 128), 0)
        i16 = lane8 & 15
        first_m = [8 * v + srow > i16 for v in range(2)]
        last_m = [8 * v + srow <= i16 for v in range(2)]
        blkid = lane8 >> 4
        blkm = [blkid == s for s in range(8)]
        blkge = [blkid >= s for s in range(8)]
        bit = [((blkid >> k) & 1) == 1 for k in range(3)]
        zero8 = jnp.zeros((8, 128), U32)
        neg8 = jnp.full((8, 128), NEG, F32)

        def st_a(b, h):
            nneg = max(0, 256 - 128 * b) if first else 0
            tmin = max(0, nneg - 112)
            qv = qt_s[8 * h:8 * h + 8, 128 * b:128 * b + 128]
            parts = [jnp.where(blkm[(s - h) % 8], qv, zero8) for s in range(8)]
            w = pltpu.bitcast(jnp.concatenate(parts, axis=0), BF)
            row0 = blk * (T // 2) + 64 * b - 72
            if tmin == 0:
                cuts = QK_CUTS
            elif tmin == 16:
                cuts = CUTS1
            else:
                cuts = CUTS0
            sv = {}
            for a_, b_ in zip(cuts[:-1], cuts[1:]):
                kc = k4_s[h, pl.ds(pl.multiple_of(row0 + a_ // 2, 8), (b_ - a_) // 2), :]
                sc = jnp.dot(pltpu.bitcast(kc, BF), w, preferred_element_type=F32)
                for v in range((b_ - a_) // 8):
                    sv[a_ // 8 + v] = sc[8 * v:8 * v + 8]
            for v in sorted(sv):
                if v < 2:
                    sv[v] = jnp.where(first_m[v], sv[v], neg8)
                elif v >= 32:
                    sv[v] = jnp.where(last_m[v - 32], sv[v], neg8)
                if 8 * v < nneg:
                    smin = -((8 * v - nneg) // 16)
                    sv[v] = jnp.where(blkge[smin], sv[v], neg8)
            vs = sorted(sv)
            m0, m1 = sv[vs[0]], sv[vs[1]]
            for v in vs[2::2]:
                m0 = jnp.maximum(m0, sv[v])
                m1 = jnp.maximum(m1, sv[v + 1])
            m = jnp.max(jnp.maximum(m0, m1), axis=0, keepdims=True)
            return jnp.broadcast_to(m, (8, 128)), sv

        def st_b(b, h, st):
            m, sv = st
            c0 = max(0, 2 - b) if first else 0
            lv = [{}, {}, {}]
            outv = []

            def sel(mk, a, c):
                if a is None and c is None:
                    return None
                return jnp.where(mk, zero8 if a is None else a, zero8 if c is None else c)

            l0 = l1 = None
            for v in range(24):
                if v < 17 and 2 * v in sv:
                    a = jnp.exp2(sv[2 * v] - m)
                    c = jnp.exp2(sv[2 * v + 1] - m)
                    l0 = a if l0 is None else l0 + a
                    l1 = c if l1 is None else l1 + c
                    lv[0][v] = _pack_pairs(a, c)
                if v < 18:
                    lv[1][v] = sel(bit[0], lv[0].get(v - 1), lv[0].get(v))
                if v < 20:
                    lv[2][v] = sel(bit[1], lv[1].get(v - 2), lv[1].get(v))
                if v >= 8 * c0:
                    o = sel(bit[2], lv[2].get(v - 4), lv[2].get(v))
                    outv.append(zero8 if o is None else o)
            l_s[h:h + 1, 128 * b:128 * b + 128] = jnp.sum(l0 + l1, axis=0, keepdims=True)
            return outv

        def st_c(b, h, outv):
            c0 = max(0, 2 - b) if first else 0
            pfull = pltpu.bitcast(jnp.concatenate(outv, axis=0), BF)
            tile0 = blk * (T // 128) + b - 2
            vt = jnp.concatenate([vt_s[tile0 + c, 8 * h:8 * h + 8, :] for c in range(c0, 3)], axis=1)
            o = jnp.dot(pltpu.bitcast(vt, BF), pfull, preferred_element_type=F32)
            ot_s[16 * h:16 * h + 16, 128 * b:128 * b + 128] = o

        items = [(b, h) for b in range(T // 128) for h in range(H)]
        n = len(items)
        sa, sb = {}, {}
        da, db = (DA0, DB0) if first else (DA, DB)
        for t in range(n + da + db):
            if t < n:
                sa[t] = st_a(*items[t])
            if fillers is not None and t in fillers:
                for f in fillers[t]:
                    f()
            u = t - da
            if 0 <= u < n:
                sb[u] = st_b(*items[u], sa.pop(u))
            w = t - da - db
            if 0 <= w < n:
                st_c(*items[w], sb.pop(w))

    def attn_proj(lo, hi):
        rl = 1.0 / l_s[:, lo:hi]
        parts = [ot_s[16 * h:16 * h + 16, lo:hi] * rl[h:h + 1, :] for h in range(H)]
        o = jnp.concatenate(parts, axis=0).T.astype(BF)
        return jnp.dot(o, wo_v[...], preferred_element_type=F32)

    def ln2(blk, z, lo, hi):
        r0 = pl.multiple_of(blk * T + lo, 128)
        g2 = 1.0 + modrow(4)
        sh = modrow(3)
        ga = modrow(2)
        for r in range(0, hi - lo, LNR):
            x1 = x_v[pl.ds(r0 + r, LNR), :].astype(F32) + ga * z[r:r + LNR]
            x1_s[lo + r:lo + r + LNR, :] = x1
            h2 = _layernorm(x1) * g2 + sh
            h2_s[lo + r:lo + r + LNR, :] = h2.astype(BF)

    def ffn_up():
        a = jnp.dot(h2_s[...], w1_v[...], preferred_element_type=F32)
        a_s[...] = jnp.maximum(a, 0.0).astype(BF)

    def ffn_down(res_ref, rlo, lo, hi, c0=0, c1=D):
        y = jnp.dot(a_s[lo:hi, :], w2_v[:, c0:c1], preferred_element_type=F32)
        gb = mod_s[0:1, 5 * D + c0:5 * D + c1]
        out_ref[lo:hi, c0:c1] = (res_ref[rlo:rlo + hi - lo, c0:c1] + gb * y).astype(out_ref.dtype)

    HT = T // 2

    def front(blk):
        q_part()
        k_part(blk)
        v_part(blk)

    @pl.when(pid == 0)
    @jax.named_scope("first")
    def _():
        for cpy in (c_copy, x_copy(0), wma_copy, wk_copy, wq_copy, x_copy(1), wv_copy, wo_copy,
                    wmb_copy, wmc_copy, w1_copy, x_copy(2), w2_copy):
            cpy.start()
        for i in range(3, NBLK):
            x_copy(i).start()
        k_s[0:64, :] = jnp.zeros((64, D), U32)
        c_copy.wait()
        x_copy(0).wait()
        if PRELN:
            ln1_pre(0)
        wma_copy.wait()
        mod_part(0, 2 * D)
        ln1(0, hn0_s, hp0_s, PRELN)
        wk_copy.wait()
        k_part(0, hn0_s)
        wq_copy.wait()
        transpose_weight(wq_v, wqt_s)
        q_part(hn0_s)
        k4_build(0)
        x_copy(1).wait()
        wv_copy.wait()
        transpose_weight(wv_v, wvt_s)
        v_part(0, hp0_s)
        ln1(1)
        k_part(1)
        v_part(1)
        wo_copy.wait()
        wmb_copy.wait()
        if MODB == 0:
            mod_part(2 * D, 5 * D)
        attention(0, True)
        if MODB == 1:
            mod_part(2 * D, 5 * D)
        if QPOS == 0:
            q_part()
        z = attn_proj(0, T)
        if QPOS == 1:
            q_part()
        if K8POS == 0:
            k4_build(1)
        ln2(0, z, 0, T)
        wmc_copy.wait()
        w1_copy.wait()
        if K8POS == 1:
            k4_build(1)
        if MODC == 0:
            mod_part(5 * D, 6 * D)
        ffn_up()
        if MODC == 1:
            mod_part(5 * D, 6 * D)
        if K8POS == 2:
            k4_build(1)

    @pl.when((pid >= 1) & (pid < NBLK - 1))
    def _():
        x_copy(pid + 1).wait()

    pl.when(pid == 1)(w2_copy.wait)

    def mid(has_next):
        if has_next and LN1POS == 0:
            ln1(pid + 1)
        fill = {FILL_T0: [lambda: ffn_down(x1_s, 0, 0, HT)]}
        attention(pid, False, fill)
        if has_next and LN1POS == 1:
            ln1(pid + 1)
        z = attn_proj(0, T)
        x1c_s[...] = x1_s[HT:T, :]
        ffn_down(x1c_s, 0, HT, T)
        if has_next and FRONTPOS == 0:
            front(pid + 1)
        ln2(pid, z, 0, T)
        if has_next and FRONTPOS == 1:
            front(pid + 1)
        ffn_up()
        if has_next:
            k4_build(pid + 1)

    @pl.when((pid >= 1) & (pid < NBLK - 1))
    @jax.named_scope("mid")
    def _():
        mid(True)

    @pl.when(pid == NBLK - 1)
    @jax.named_scope("mid7")
    def _():
        mid(False)

    @pl.when(pid == NBLK)
    @jax.named_scope("last")
    def _():
        ffn_down(x1_s, 0, 0, T)


@jax.jit
def pallas_adaLN_cond__sliding_block__dense_activation_relu__prompt_kernel(
    A_x: jax.Array,
    A_wqkv: jax.Array,
    A_wo: jax.Array,
    B_x: jax.Array,
    B_w1: jax.Array,
    B_w2: jax.Array,
    c: jax.Array,
    w_mod: jax.Array,
):
    del B_x
    x = A_x.reshape(S, D)
    any_spec = pl.BlockSpec(memory_space=pl.ANY)
    scratch = [
        pltpu.VMEM((S, D), BF),
        pltpu.VMEM((D, D), BF),
        pltpu.VMEM((D, D), BF),
        pltpu.VMEM((D, D), BF),
        pltpu.VMEM((D, D), BF),
        pltpu.VMEM((D, DFF), BF),
        pltpu.VMEM((DFF, D), BF),
        pltpu.VMEM((1, D), BF),
        pltpu.VMEM((D, 6 * D), BF),
        pltpu.VMEM((D, D), BF),
        pltpu.VMEM((D, D), BF),
        pltpu.VMEM((8, 6 * D), F32),
        pltpu.VMEM((T, D), BF),
        pltpu.VMEM((T // 2, D), U32),
        pltpu.VMEM((T, D), BF),
        pltpu.VMEM((T // 2, D), U32),
        pltpu.VMEM((S // 2 + 64, D), U32),
        pltpu.VMEM((H, S // 2, 128), U32),
        pltpu.VMEM((S // 128, D // 2, 128), U32),
        pltpu.VMEM((D // 2, T), U32),
        pltpu.VMEM((D, T), F32),
        pltpu.VMEM((H, T), F32),
        pltpu.VMEM((T, D), F32),
        pltpu.VMEM((T, D), BF),
        pltpu.VMEM((T // 2, D), F32),
        pltpu.VMEM((T, DFF), BF),
        pltpu.SemaphoreType.DMA((NSEM,)),
    ]
    out = pl.pallas_call(
        _kernel,
        grid=(NBLK + 1,),
        in_specs=[any_spec] * 7,
        out_specs=pl.BlockSpec((T, D), lambda i: (jnp.maximum(i - 1, 0), 0)),
        out_shape=jax.ShapeDtypeStruct((S, D), BF),
        scratch_shapes=scratch,
        compiler_params=pltpu.CompilerParams(
            dimension_semantics=("arbitrary",),
            vmem_limit_bytes=100 * 1024 * 1024),
    )(x, A_wqkv, A_wo, B_w1, B_w2, c, w_mod)
    return out.reshape(1, S, D)
```

```python
import jax
import jax.numpy as jnp
import jax.experimental.pallas as pl
import jax.experimental.pallas.tpu as pltpu

F32 = jnp.float32
BF = jnp.bfloat16
U32 = jnp.uint32

S = 2048
D = 512
H = 32
DFF = 1792
T = 256
NBLK = S // T
EPS = 1e-5
QSCALE = 0.25 * 1.4426950408889634
NEG = -1e30
NT = (((1,), (1,)), ((), ()))

W2WAIT = 1
LNR = 16
LN1POS = 1
FRONTPOS = 0
FILL_N = 1
FILL_T0 = 64
FILL_DT = 16
TAIL0 = 0
PRELN = 1
K8POS = 0
MODC = 1
QPOS = 1
MODB = 0
CUTS0 = (144,208,272)
CUTS1 = (16,80,144,208,272)
W1POS = 1
ORDER = 'c0_c1_c2_c3_B_p0_p1_p2'
ORDER0 = 'c0_c1_c2_c3_B_p0_p1_p2'
WB = 1
FULLDOWN = 1
ILV0 = 0
DA0 = 4
DB0 = 3
DA = 2
DB = 2
QK_CUTS = (0,64,128,192,272)

(SEM_C, SEM_WMA, SEM_WQ, SEM_WV, SEM_WK, SEM_WMB, SEM_WO, SEM_W1, SEM_W2, SEM_WMC) = range(10)
SEM_X0 = 10
SEM_O0 = SEM_X0 + NBLK
NSEM = SEM_O0 + NBLK + 2
LASTCUT = (0,128,192,256)
O6POS = 0


def _u32(x):
    return x if x.dtype == U32 else pltpu.bitcast(x, U32)


def _pack_pairs(a, b):
    return _u32(pltpu.pack_elementwise([a, b], packed_dtype=BF))


def _layernorm(x):
    mu = jnp.mean(x, axis=-1, keepdims=True)
    xc = x - mu
    var = jnp.mean(xc * xc, axis=-1, keepdims=True)
    return xc * jax.lax.rsqrt(var + EPS)


def _kernel(x_hbm, wqkv_hbm, wo_hbm, w1_hbm, w2_hbm, c_hbm, wmod_hbm, out_hbm,
            x_v, wq_v, wk_v, wv_v, wo_v, w1_v, w2_v, c_v, wmod_v,
            wqt_s, wvt_s, mod_s, hn_s, hp_s, hn0_s, hp0_s, k_s, k4_s, vt_s, qt_s, ot_s, l_s,
            x1_s, h2_s, x1c_s, a_s, o_s, msk_s, sems):
    pid = pl.program_id(0)

    def cp(src, dst, slot):
        return pltpu.make_async_copy(src, dst, sems.at[slot])

    def x_copy(i):
        return cp(x_hbm.at[pl.ds(i * T, T), :], x_v.at[pl.ds(i * T, T), :], SEM_X0 + i)

    def o_copy(r0, n, slot):
        return cp(o_s.at[pl.ds(r0, n), :], out_hbm.at[pl.ds(r0, n), :], SEM_O0 + slot)

    c_copy = cp(c_hbm, c_v, SEM_C)
    wma_copy = cp(wmod_hbm.at[:, pl.ds(0, 2 * D)], wmod_v.at[:, pl.ds(0, 2 * D)], SEM_WMA)
    wmb_copy = cp(wmod_hbm.at[:, pl.ds(2 * D, 3 * D)], wmod_v.at[:, pl.ds(2 * D, 3 * D)], SEM_WMB)
    wmc_copy = cp(wmod_hbm.at[:, pl.ds(5 * D, D)], wmod_v.at[:, pl.ds(5 * D, D)], SEM_WMC)
    wq_copy = cp(wqkv_hbm.at[:, pl.ds(0, D)], wq_v, SEM_WQ)
    wk_copy = cp(wqkv_hbm.at[:, pl.ds(D, D)], wk_v, SEM_WK)
    wv_copy = cp(wqkv_hbm.at[:, pl.ds(2 * D, D)], wv_v, SEM_WV)
    wo_copy = cp(wo_hbm, wo_v, SEM_WO)
    w1_copy = cp(w1_hbm, w1_v, SEM_W1)
    w2_copy = cp(w2_hbm, w2_v, SEM_W2)

    def mod_part(lo, hi):
        cf = c_v[...].astype(F32)
        sc = cf * (1.0 / (1.0 + jnp.exp(-cf)))
        sc = jnp.broadcast_to(sc, (16, D)).astype(BF)
        m = jnp.dot(sc, wmod_v[:, lo:hi], preferred_element_type=F32)
        mod_s[:, lo:hi] = m[0:8]

    def modrow(k):
        return mod_s[0:1, k * D:(k + 1) * D]

    def transpose_weight(w_v, wt_s):
        r = jax.lax.broadcasted_iota(jnp.int32, (128, 128), 0)
        f = jax.lax.broadcasted_iota(jnp.int32, (128, 128), 1)
        src = (r & ~15) + 2 * (r & 7) + ((r >> 3) & 1)
        pm = jnp.where(f == src, 1.0, 0.0).astype(BF)
        for ft in range(4):
            res = jax.lax.dot_general(pm, w_v[:, 128 * ft:128 * ft + 128], NT,
                                      preferred_element_type=F32)
            wt_s[128 * ft:128 * ft + 128, :] = res.astype(BF)

    def ln1_pre(blk):
        for r in range(0, T, LNR):
            x1_s[r:r + LNR, :] = _layernorm(x_v[blk * T + r:blk * T + r + LNR, :].astype(F32))

    def ln1(blk, hn_s=hn_s, hp_s=hp_s, pre=False):
        r0 = pl.multiple_of(blk * T, T)
        g1 = 1.0 + modrow(1)
        sh = modrow(0)
        for r in range(0, T, LNR):
            if pre:
                xn = x1_s[r:r + LNR, :]
            else:
                xn = _layernorm(x_v[pl.ds(r0 + r, LNR), :].astype(F32))
            h = xn * g1 + sh
            hn_s[r:r + LNR, :] = h.astype(BF)
            for g in range(LNR // 16):
                hp_s[r // 2 + 8 * g:r // 2 + 8 * g + 8, :] = _pack_pairs(
                    h[16 * g:16 * g + 8], h[16 * g + 8:16 * g + 16])

    def q_part(hn_s=hn_s):
        qt = jax.lax.dot_general(wqt_s[...], hn_s[...], NT, preferred_element_type=F32) * QSCALE
        for h in range(H):
            qt_s[8 * h:8 * h + 8, :] = _pack_pairs(qt[16 * h:16 * h + 8], qt[16 * h + 8:16 * h + 16])

    def k_part(blk, hn_s=hn_s):
        k = jnp.dot(hn_s[...], wk_v[...], preferred_element_type=F32)
        r0 = pl.multiple_of(blk * (T // 2) + 64, 64)
        k_s[pl.ds(r0, T // 2), :] = _u32(k.astype(BF))

    def v_part(blk, hp_s=hp_s):
        hp = pltpu.bitcast(hp_s[...], BF)
        vt = jax.lax.dot_general(wvt_s[...], hp, NT, preferred_element_type=F32)
        for b in range(T // 128):
            pk = [_pack_pairs(vt[16 * h:16 * h + 8, 128 * b:128 * b + 128],
                              vt[16 * h + 8:16 * h + 16, 128 * b:128 * b + 128]) for h in range(H)]
            vt_s[blk * (T // 128) + b] = jnp.concatenate(pk, axis=0)

    def k4_build(blk):
        lane = jax.lax.broadcasted_iota(jnp.int32, (8, 128), 1)
        bit = [((lane >> (4 + k)) & 1) == 1 for k in range(3)]
        src0 = blk * (T // 2) + 8
        dst0 = blk * (T // 2)
        for g in range(4):
            xs = {}

            def x(w, g=g, xs=xs):
                if w not in xs:
                    xs[w] = k_s[pl.ds(pl.multiple_of(src0 + 8 * w, 8), 8), 128 * g:128 * g + 128]
                return xs[w]

            for u in range(T // 16):
                f = [x(u)] + [pltpu.roll(x(u + d), 16 * d, 1) for d in range(1, 8)]
                for k in range(3):
                    f = [jnp.where(bit[k], f[(m + (1 << k)) % 8], f[m]) for m in range(8)]
                for hh in range(8):
                    k4_s[8 * g + hh, pl.ds(pl.multiple_of(dst0 + 8 * u, 8), 8), :] = f[(-hh) % 8]

    def attention(blk, first, fillers=None):
        lane8 = jax.lax.broadcasted_iota(jnp.int32, (8, 128), 1)
        srow = jax.lax.broadcasted_iota(jnp.int32, (8, 128), 0)
        i16 = lane8 & 15
        first_m = [8 * v + srow > i16 for v in range(2)]
        last_m = [8 * v + srow <= i16 for v in range(2)]
        blkid = lane8 >> 4
        blkm = [blkid == s for s in range(8)]
        blkge = [blkid >= s for s in range(8)]
        bit = [((blkid >> k) & 1) == 1 for k in range(3)]
        zero8 = jnp.zeros((8, 128), U32)
        neg8 = jnp.full((8, 128), NEG, F32)

        def st_a0(b, h):
            nneg = max(0, 256 - 128 * b) if first else 0
            tmin = max(0, nneg - 112)
            qv = qt_s[8 * h:8 * h + 8, 128 * b:128 * b + 128]
            if WB == 0:
                parts = [jnp.where(blkm[(s - h) % 8], qv, zero8) for s in range(8)]
            elif WB == 1:
                lvl = [qv]
                for k in (2, 1, 0):
                    lvl = [x for y in lvl
                           for x in (jnp.where(bit[k], zero8, y), jnp.where(bit[k], y, zero8))]
                parts = [lvl[(s - h) % 8] for s in range(8)]
            else:
                parts = [qv & msk_s[8 * ((s - h) % 8):8 * ((s - h) % 8) + 8, :] for s in range(8)]
            w = pltpu.bitcast(jnp.concatenate(parts, axis=0), BF)
            if tmin == 0:
                cuts = QK_CUTS
            elif tmin == 16:
                cuts = CUTS1
            else:
                cuts = CUTS0
            return dict(w=w, cuts=list(zip(cuts[:-1], cuts[1:])), sv={}, nneg=nneg)

        def st_a1(b, h, st, j):
            if j >= len(st["cuts"]):
                return
            a_, b_ = st["cuts"][j]
            row0 = blk * (T // 2) + 64 * b - 72
            kc = k4_s[h, pl.ds(pl.multiple_of(row0 + a_ // 2, 8), (b_ - a_) // 2), :]
            sc = jnp.dot(pltpu.bitcast(kc, BF), st["w"], preferred_element_type=F32)
            for v in range((b_ - a_) // 8):
                st["sv"][a_ // 8 + v] = sc[8 * v:8 * v + 8]

        def st_a2(b, h, st):
            sv, nneg = st["sv"], st["nneg"]
            for v in sorted(sv):
                if v < 2:
                    sv[v] = jnp.where(first_m[v], sv[v], neg8)
                elif v >= 32:
                    sv[v] = jnp.where(last_m[v - 32], sv[v], neg8)
                if 8 * v < nneg:
                    smin = -((8 * v - nneg) // 16)
                    sv[v] = jnp.where(blkge[smin], sv[v], neg8)
            vs = sorted(sv)
            m0, m1 = sv[vs[0]], sv[vs[1]]
            for v in vs[2::2]:
                m0 = jnp.maximum(m0, sv[v])
                m1 = jnp.maximum(m1, sv[v + 1])
            m = jnp.max(jnp.maximum(m0, m1), axis=0, keepdims=True)
            return jnp.broadcast_to(m, (8, 128)), sv

        def st_b(b, h, st):
            m, sv = st
            c0 = max(0, 2 - b) if first else 0
            lv = [{}, {}, {}]
            outv = []

            def sel(mk, a, c):
                if a is None and c is None:
                    return None
                return jnp.where(mk, zero8 if a is None else a, zero8 if c is None else c)

            l0 = l1 = None
            for v in range(24):
                if v < 17 and 2 * v in sv:
                    a = jnp.exp2(sv[2 * v] - m)
                    c = jnp.exp2(sv[2 * v + 1] - m)
                    l0 = a if l0 is None else l0 + a
                    l1 = c if l1 is None else l1 + c
                    lv[0][v] = _pack_pairs(a, c)
                if v < 18:
                    lv[1][v] = sel(bit[0], lv[0].get(v - 1), lv[0].get(v))
                if v < 20:
                    lv[2][v] = sel(bit[1], lv[1].get(v - 2), lv[1].get(v))
                if v >= 8 * c0:
                    o = sel(bit[2], lv[2].get(v - 4), lv[2].get(v))
                    outv.append(zero8 if o is None else o)
            l_s[h:h + 1, 128 * b:128 * b + 128] = jnp.sum(l0 + l1, axis=0, keepdims=True)
            return outv

        def st_c1(b, h, outv, c, acc):
            c0 = max(0, 2 - b) if first else 0
            if c < c0:
                return acc
            tile0 = blk * (T // 128) + b - 2
            pt = pltpu.bitcast(jnp.concatenate(outv[8 * (c - c0):8 * (c - c0) + 8], axis=0), BF)
            vt = vt_s[tile0 + c, 8 * h:8 * h + 8, :]
            o = jnp.dot(pltpu.bitcast(vt, BF), pt, preferred_element_type=F32)
            return o if acc is None else acc + o

        items = [(b, h) for b in range(T // 128) for h in range(H)]
        if first and ILV0:
            items = [(b, h) for h in range(H) for b in range(T // 128)]
        n = len(items)
        sa, sb = {}, {}
        da, db = (DA0, DB0) if first else (DA, DB)
        for t in range(n + da + db):
            w = t - da - db
            st = st_a0(*items[t]) if t < n else None
            acc = None
            for o in (ORDER0 if first else ORDER).split("_"):
                if o[0] == "c" and st is not None:
                    st_a1(*items[t], st, int(o[1]))
                if o[0] == "p" and 0 <= w < n:
                    acc = st_c1(*items[w], sb[w], int(o[1]), acc)
                if o == "B":
                    u = t - da
                    if 0 <= u < n:
                        sb[u] = st_b(*items[u], sa.pop(u))
            if st is not None:
                sa[t] = st_a2(*items[t], st)
            if 0 <= w < n:
                b, h = items[w]
                sb.pop(w)
                ot_s[16 * h:16 * h + 16, 128 * b:128 * b + 128] = acc
            if fillers is not None and t in fillers:
                for f in fillers[t]:
                    f()

    def attn_proj(lo, hi):
        rl = 1.0 / l_s[:, lo:hi]
        parts = [ot_s[16 * h:16 * h + 16, lo:hi] * rl[h:h + 1, :] for h in range(H)]
        o = jnp.concatenate(parts, axis=0).T.astype(BF)
        return jnp.dot(o, wo_v[...], preferred_element_type=F32)

    def ln2(blk, z, lo, hi):
        r0 = pl.multiple_of(blk * T + lo, 128)
        g2 = 1.0 + modrow(4)
        sh = modrow(3)
        ga = modrow(2)
        for r in range(0, hi - lo, LNR):
            x1 = x_v[pl.ds(r0 + r, LNR), :].astype(F32) + ga * z[r:r + LNR]
            x1_s[lo + r:lo + r + LNR, :] = x1
            h2 = _layernorm(x1) * g2 + sh
            h2_s[lo + r:lo + r + LNR, :] = h2.astype(BF)

    def ffn_up():
        a = jnp.dot(h2_s[...], w1_v[...], preferred_element_type=F32)
        a_s[...] = jnp.maximum(a, 0.0).astype(BF)

    def ffn_down(blk, res_ref, rlo, lo, hi):
        y = jnp.dot(a_s[lo:hi, :], w2_v[...], preferred_element_type=F32)
        r0 = pl.multiple_of(blk * T + lo, 64)
        o_s[pl.ds(r0, hi - lo), :] = (
            res_ref[rlo:rlo + hi - lo, :] + modrow(5) * y).astype(BF)

    HT = T // 2

    def front(blk):
        q_part()
        k_part(blk)
        v_part(blk)

    @pl.when(pid == 0)
    @jax.named_scope("first")
    def _():
        for cpy in (c_copy, x_copy(0), wma_copy, wk_copy, wq_copy, x_copy(1), wv_copy, wo_copy,
                    wmb_copy, wmc_copy, w1_copy, x_copy(2), w2_copy):
            cpy.start()
        for i in range(3, NBLK):
            x_copy(i).start()
        k_s[0:64, :] = jnp.zeros((64, D), U32)
        mrow = jax.lax.broadcasted_iota(jnp.int32, (64, 128), 0) >> 3
        mcol = jax.lax.broadcasted_iota(jnp.int32, (64, 128), 1) >> 4
        msk_s[...] = jnp.where(mrow == mcol, jnp.uint32(0xFFFFFFFF), jnp.uint32(0))
        c_copy.wait()
        x_copy(0).wait()
        if PRELN:
            ln1_pre(0)
        wma_copy.wait()
        mod_part(0, 2 * D)
        ln1(0, hn0_s, hp0_s, PRELN)
        wk_copy.wait()
        k_part(0, hn0_s)
        wq_copy.wait()
        transpose_weight(wq_v, wqt_s)
        q_part(hn0_s)
        k4_build(0)
        x_copy(1).wait()
        wv_copy.wait()
        transpose_weight(wv_v, wvt_s)
        v_part(0, hp0_s)
        ln1(1)
        k_part(1)
        v_part(1)
        wo_copy.wait()
        wmb_copy.wait()
        if MODB == 0:
            mod_part(2 * D, 5 * D)
        attention(0, True)
        if MODB == 1:
            mod_part(2 * D, 5 * D)
        if QPOS == 0:
            q_part()
        z = attn_proj(0, T)
        if QPOS == 1:
            q_part()
        if K8POS == 0:
            k4_build(1)
        ln2(0, z, 0, T)
        wmc_copy.wait()
        w1_copy.wait()
        if K8POS == 1:
            k4_build(1)
        if MODC == 0:
            mod_part(5 * D, 6 * D)
        ffn_up()
        if MODC == 1:
            mod_part(5 * D, 6 * D)
        if K8POS == 2:
            k4_build(1)

    @pl.when((pid >= 1) & (pid < NBLK - 1))
    def _():
        x_copy(pid + 1).wait()

    pl.when(pid == 1)(w2_copy.wait)

    @pl.when(pid >= 2)
    def _():
        o_copy((pid - 2) * T, T, pid - 2).start()

    def mid(has_next):
        full = FULLDOWN and has_next
        if has_next and LN1POS == 0:
            ln1(pid + 1)
        fill = {FILL_T0: [lambda: ffn_down(pid - 1, x1_s, 0, 0, T if full else HT)]}
        attention(pid, False, fill)
        if has_next and LN1POS == 1:
            ln1(pid + 1)
        if has_next and FRONTPOS >= 2:
            k_part(pid + 1)
        if has_next and FRONTPOS == 3:
            k4_build(pid + 1)
        if has_next and FRONTPOS == 4:
            v_part(pid + 1)
        z = attn_proj(0, T)
        if not full:
            x1c_s[...] = x1_s[HT:T, :]
            ffn_down(pid - 1, x1c_s, 0, HT, T)
        if not has_next and O6POS == 0:
            o_copy((NBLK - 2) * T, T, NBLK - 2).start()
        if has_next and FRONTPOS == 0:
            front(pid + 1)
        if has_next and FRONTPOS >= 2:
            q_part()
            if FRONTPOS != 4:
                v_part(pid + 1)
        ln2(pid, z, 0, T)
        if has_next and FRONTPOS == 1:
            front(pid + 1)
        ffn_up()
        if not has_next and O6POS == 1:
            o_copy((NBLK - 2) * T, T, NBLK - 2).start()
        if has_next and FRONTPOS != 3:
            k4_build(pid + 1)

    @pl.when((pid >= 1) & (pid < NBLK - 1))
    @jax.named_scope("mid")
    def _():
        mid(True)

    @pl.when(pid == NBLK - 1)
    @jax.named_scope("mid7")
    def _():
        mid(False)
        last = []
        for j, (lo, hi) in enumerate(zip(LASTCUT[:-1], LASTCUT[1:])):
            ffn_down(NBLK - 1, x1_s, lo, lo, hi)
            last.append(o_copy((NBLK - 1) * T + lo, hi - lo, NBLK - 1 + j))
            last[-1].start()
        for i in range(NBLK - 1):
            o_copy(i * T, T, i).wait()
        for cpy in last:
            cpy.wait()


@jax.jit
def pallas_adaLN_cond__sliding_block__dense_activation_relu__prompt_kernel(
    A_x: jax.Array,
    A_wqkv: jax.Array,
    A_wo: jax.Array,
    B_x: jax.Array,
    B_w1: jax.Array,
    B_w2: jax.Array,
    c: jax.Array,
    w_mod: jax.Array,
):
    del B_x
    x = A_x.reshape(S, D)
    any_spec = pl.BlockSpec(memory_space=pl.ANY)
    scratch = [
        pltpu.VMEM((S, D), BF),
        pltpu.VMEM((D, D), BF),
        pltpu.VMEM((D, D), BF),
        pltpu.VMEM((D, D), BF),
        pltpu.VMEM((D, D), BF),
        pltpu.VMEM((D, DFF), BF),
        pltpu.VMEM((DFF, D), BF),
        pltpu.VMEM((1, D), BF),
        pltpu.VMEM((D, 6 * D), BF),
        pltpu.VMEM((D, D), BF),
        pltpu.VMEM((D, D), BF),
        pltpu.VMEM((8, 6 * D), F32),
        pltpu.VMEM((T, D), BF),
        pltpu.VMEM((T // 2, D), U32),
        pltpu.VMEM((T, D), BF),
        pltpu.VMEM((T // 2, D), U32),
        pltpu.VMEM((S // 2 + 64, D), U32),
        pltpu.VMEM((H, S // 2, 128), U32),
        pltpu.VMEM((S // 128, D // 2, 128), U32),
        pltpu.VMEM((D // 2, T), U32),
        pltpu.VMEM((D, T), F32),
        pltpu.VMEM((H, T), F32),
        pltpu.VMEM((T, D), F32),
        pltpu.VMEM((T, D), BF),
        pltpu.VMEM((T // 2, D), F32),
        pltpu.VMEM((T, DFF), BF),
        pltpu.VMEM((S, D), BF),
        pltpu.VMEM((64, 128), U32),
        pltpu.SemaphoreType.DMA((NSEM,)),
    ]
    out = pl.pallas_call(
        _kernel,
        grid=(NBLK,),
        in_specs=[any_spec] * 7,
        out_specs=any_spec,
        out_shape=jax.ShapeDtypeStruct((S, D), BF),
        scratch_shapes=scratch,
        compiler_params=pltpu.CompilerParams(
            dimension_semantics=("arbitrary",),
            vmem_limit_bytes=100 * 1024 * 1024),
    )(x, A_wqkv, A_wo, B_w1, B_w2, c, w_mod)
    return out.reshape(1, S, D)
```

```python
import jax
import jax.numpy as jnp
import jax.experimental.pallas as pl
import jax.experimental.pallas.tpu as pltpu

F32 = jnp.float32
BF = jnp.bfloat16
U32 = jnp.uint32

S = 2048
D = 512
H = 32
DFF = 1792
T = 256
HT = T // 2
HD = D // 2
NBLK = S // T
EPS = 1e-5
QSCALE = 0.25 * 1.4426950408889634
NEG = -1e30
NT = (((1,), (1,)), ((), ()))

LNR = 16
QK_CUTS = (0, 64, 128, 192, 272)
CUTS0 = (144, 208, 272)
CUTS1 = (16, 80, 144, 208, 272)
DA, DB = 2, 2
DA0, DB0 = 4, 3
LASTCUT = (0, 128, 192, 256)

(SEM_C, SEM_WMA, SEM_WQ, SEM_WV, SEM_WKA, SEM_WKB, SEM_WMB, SEM_WO, SEM_W1, SEM_W2,
 SEM_WMC) = range(11)
SEM_X0 = 11
SEM_O0 = SEM_X0 + NBLK
NSEM = SEM_O0 + NBLK - 1 + len(LASTCUT) - 1


def _u32(x):
    return x if x.dtype == U32 else pltpu.bitcast(x, U32)


def _pack_pairs(a, b):
    return _u32(pltpu.pack_elementwise([a, b], packed_dtype=BF))


def _layernorm(x):
    mu = jnp.mean(x, axis=-1, keepdims=True)
    xc = x - mu
    var = jnp.mean(xc * xc, axis=-1, keepdims=True)
    return xc * jax.lax.rsqrt(var + EPS)


def _kernel(x_hbm, wqkv_hbm, wo_hbm, w1_hbm, w2_hbm, c_hbm, wmod_hbm, out_hbm,
            x_v, wq_v, wk_v, wv_v, wo_v, w1_v, w2_v, c_v, wmod_v,
            wqt_s, wvt_s, mod_s, hn_s, hp_s, hn0_s, hp0_s, k_s, k8_s, vt_s, qt_s, ot_s, l_s,
            x1_s, h2_s, x1c_s, a_s, o_s, sems):
    pid = pl.program_id(0)

    def cp(src, dst, slot):
        return pltpu.make_async_copy(src, dst, sems.at[slot])

    def x_copy(i):
        return cp(x_hbm.at[pl.ds(i * T, T), :], x_v.at[pl.ds(i * T, T), :], SEM_X0 + i)

    def o_copy(r0, n, slot):
        return cp(o_s.at[pl.ds(r0, n), :], out_hbm.at[pl.ds(r0, n), :], SEM_O0 + slot)

    c_copy = cp(c_hbm, c_v, SEM_C)
    wma_copy = cp(wmod_hbm.at[:, pl.ds(0, 2 * D)], wmod_v.at[:, pl.ds(0, 2 * D)], SEM_WMA)
    wmb_copy = cp(wmod_hbm.at[:, pl.ds(2 * D, 3 * D)], wmod_v.at[:, pl.ds(2 * D, 3 * D)], SEM_WMB)
    wmc_copy = cp(wmod_hbm.at[:, pl.ds(5 * D, D)], wmod_v.at[:, pl.ds(5 * D, D)], SEM_WMC)
    wq_copy = cp(wqkv_hbm.at[:, pl.ds(0, D)], wq_v, SEM_WQ)
    wka_copy = cp(wqkv_hbm.at[:, pl.ds(D, HD)], wk_v.at[:, pl.ds(0, HD)], SEM_WKA)
    wkb_copy = cp(wqkv_hbm.at[:, pl.ds(D + HD, HD)], wk_v.at[:, pl.ds(HD, HD)], SEM_WKB)
    wv_copy = cp(wqkv_hbm.at[:, pl.ds(2 * D, D)], wv_v, SEM_WV)
    wo_copy = cp(wo_hbm, wo_v, SEM_WO)
    w1_copy = cp(w1_hbm, w1_v, SEM_W1)
    w2_copy = cp(w2_hbm, w2_v, SEM_W2)

    def mod_part(lo, hi):
        cf = c_v[...].astype(F32)
        sc = cf * (1.0 / (1.0 + jnp.exp(-cf)))
        sc = jnp.broadcast_to(sc, (16, D)).astype(BF)
        m = jnp.dot(sc, wmod_v[:, lo:hi], preferred_element_type=F32)
        mod_s[:, lo:hi] = m[0:8]

    def modrow(k):
        return mod_s[0:1, k * D:(k + 1) * D]

    def ln1_pre():
        for r in range(0, T, LNR):
            x1_s[r:r + LNR, :] = _layernorm(x_v[r:r + LNR, :].astype(F32))

    def ln1(blk, hn_s=hn_s, hp_s=hp_s, pre=False):
        r0 = pl.multiple_of(blk * T, T)
        g1 = 1.0 + modrow(1)
        sh = modrow(0)
        for r in range(0, T, LNR):
            if pre:
                xn = x1_s[r:r + LNR, :]
            else:
                xn = _layernorm(x_v[pl.ds(r0 + r, LNR), :].astype(F32))
            h = xn * g1 + sh
            hn_s[r:r + LNR, :] = h.astype(BF)
            for g in range(LNR // 16):
                hp_s[r // 2 + 8 * g:r // 2 + 8 * g + 8, :] = _pack_pairs(
                    h[16 * g:16 * g + 8], h[16 * g + 8:16 * g + 16])

    def q_part(hn_s=hn_s):
        qt = jax.lax.dot_general(wqt_s[...], hn_s[...], NT, preferred_element_type=F32) * QSCALE
        qt_s[...] = _u32(qt.astype(BF))

    def k_part(blk, hn_s=hn_s, lo=0, hi=D):
        k = jnp.dot(hn_s[...], wk_v[:, lo:hi], preferred_element_type=F32)
        r0 = pl.multiple_of(blk * HT + 64, 64)
        k_s[pl.ds(r0, HT), lo:hi] = _u32(k.astype(BF))

    def v_part(blk, hp_s=hp_s):
        hp = pltpu.bitcast(hp_s[...], BF)
        vt = jax.lax.dot_general(wvt_s[...], hp, NT, preferred_element_type=F32)
        for b in range(T // 128):
            vt_s[blk * (T // 128) + b] = _u32(vt[:, 128 * b:128 * b + 128].astype(BF))

    def k8_build(blk):
        lane = jax.lax.broadcasted_iota(jnp.int32, (8, 128), 1)
        bit = [((lane >> (4 + k)) & 1) == 1 for k in range(3)]
        src0 = blk * HT + 8
        dst0 = blk * HT
        for g in range(4):
            xs = {}

            def x(w, g=g, xs=xs):
                if w not in xs:
                    xs[w] = k_s[pl.ds(pl.multiple_of(src0 + 8 * w, 8), 8), 128 * g:128 * g + 128]
                return xs[w]

            for u in range(T // 16):
                f = [x(u)] + [pltpu.roll(x(u + d), 16 * d, 1) for d in range(1, 8)]
                for k in range(3):
                    f = [jnp.where(bit[k], f[(m + (1 << k)) % 8], f[m]) for m in range(8)]
                for hh in range(8):
                    k8_s[8 * g + hh, pl.ds(pl.multiple_of(dst0 + 8 * u, 8), 8), :] = f[(-hh) % 8]

    def attention(blk, first, filler=None):
        lane8 = jax.lax.broadcasted_iota(jnp.int32, (8, 128), 1)
        srow = jax.lax.broadcasted_iota(jnp.int32, (8, 128), 0)
        i16 = lane8 & 15
        first_m = [8 * v + srow > i16 for v in range(2)]
        last_m = [8 * v + srow <= i16 for v in range(2)]
        blkid = lane8 >> 4
        blkge = [blkid >= s for s in range(8)]
        bit = [((blkid >> k) & 1) == 1 for k in range(3)]
        zero8 = jnp.zeros((8, 128), U32)
        neg8 = jnp.full((8, 128), NEG, F32)

        def qk(b, h):
            nneg = max(0, 256 - 128 * b) if first else 0
            tmin = max(0, nneg - 112)
            lvl = [qt_s[8 * h:8 * h + 8, 128 * b:128 * b + 128]]
            for k in (2, 1, 0):
                lvl = [x for y in lvl
                       for x in (jnp.where(bit[k], zero8, y), jnp.where(bit[k], y, zero8))]
            w = pltpu.bitcast(jnp.concatenate([lvl[(s - h) % 8] for s in range(8)], axis=0), BF)
            cuts = QK_CUTS if tmin == 0 else (CUTS1 if tmin == 16 else CUTS0)
            sv = {}
            row0 = blk * HT + 64 * b - 72
            for a_, b_ in zip(cuts[:-1], cuts[1:]):
                kc = k8_s[h, pl.ds(pl.multiple_of(row0 + a_ // 2, 8), (b_ - a_) // 2), :]
                sc = jnp.dot(pltpu.bitcast(kc, BF), w, preferred_element_type=F32)
                for v in range((b_ - a_) // 8):
                    sv[a_ // 8 + v] = sc[8 * v:8 * v + 8]
            return sv, nneg

        def mask_max(sv, nneg):
            for v in sorted(sv):
                if v < 2:
                    sv[v] = jnp.where(first_m[v], sv[v], neg8)
                elif v >= 32:
                    sv[v] = jnp.where(last_m[v - 32], sv[v], neg8)
                if 8 * v < nneg:
                    smin = -((8 * v - nneg) // 16)
                    sv[v] = jnp.where(blkge[smin], sv[v], neg8)
            vs = sorted(sv)
            m0, m1 = sv[vs[0]], sv[vs[1]]
            for v in vs[2::2]:
                m0 = jnp.maximum(m0, sv[v])
                m1 = jnp.maximum(m1, sv[v + 1])
            m = jnp.max(jnp.maximum(m0, m1), axis=0, keepdims=True)
            return jnp.broadcast_to(m, (8, 128)), sv

        def probs(b, h, st):
            m, sv = st
            c0 = max(0, 2 - b) if first else 0
            lv = [{}, {}, {}]
            outv = []

            def sel(mk, a, c):
                if a is None and c is None:
                    return None
                return jnp.where(mk, zero8 if a is None else a, zero8 if c is None else c)

            l0 = l1 = None
            for v in range(24):
                if v < 17 and 2 * v in sv:
                    a = jnp.exp2(sv[2 * v] - m)
                    c = jnp.exp2(sv[2 * v + 1] - m)
                    l0 = a if l0 is None else l0 + a
                    l1 = c if l1 is None else l1 + c
                    lv[0][v] = _pack_pairs(a, c)
                if v < 18:
                    lv[1][v] = sel(bit[0], lv[0].get(v - 1), lv[0].get(v))
                if v < 20:
                    lv[2][v] = sel(bit[1], lv[1].get(v - 2), lv[1].get(v))
                if v >= 8 * c0:
                    o = sel(bit[2], lv[2].get(v - 4), lv[2].get(v))
                    outv.append(zero8 if o is None else o)
            l_s[h:h + 1, 128 * b:128 * b + 128] = jnp.sum(l0 + l1, axis=0, keepdims=True)
            return outv

        def pv(b, h, outv):
            c0 = max(0, 2 - b) if first else 0
            tile0 = blk * (T // 128) + b - 2
            acc = None
            for c in range(c0, 3):
                pt = pltpu.bitcast(
                    jnp.concatenate(outv[8 * (c - c0):8 * (c - c0) + 8], axis=0), BF)
                vt = vt_s[tile0 + c, 8 * h:8 * h + 8, :]
                o = jnp.dot(pltpu.bitcast(vt, BF), pt, preferred_element_type=F32)
                acc = o if acc is None else acc + o
            ot_s[16 * h:16 * h + 16, 128 * b:128 * b + 128] = acc

        items = [(b, h) for b in range(T // 128) for h in range(H)]
        n = len(items)
        sa, sb = {}, {}
        da, db = (DA0, DB0) if first else (DA, DB)
        for t in range(n + da + db):
            st = qk(*items[t]) if t < n else None
            if 0 <= t - da < n:
                sb[t - da] = probs(*items[t - da], sa.pop(t - da))
            if 0 <= t - da - db < n:
                pv(*items[t - da - db], sb.pop(t - da - db))
            if st is not None:
                sa[t] = mask_max(*st)
            if filler is not None and t == n:
                filler()

    def attn_proj():
        rl = 1.0 / l_s[...]
        parts = [ot_s[16 * h:16 * h + 16, :] * rl[h:h + 1, :] for h in range(H)]
        o = jnp.concatenate(parts, axis=0).T.astype(BF)
        return jnp.dot(o, wo_v[...], preferred_element_type=F32)

    def ln2(blk, z):
        r0 = pl.multiple_of(blk * T, T)
        g2 = 1.0 + modrow(4)
        sh = modrow(3)
        ga = modrow(2)
        for r in range(0, T, LNR):
            x1 = x_v[pl.ds(r0 + r, LNR), :].astype(F32) + ga * z[r:r + LNR]
            x1_s[r:r + LNR, :] = x1
            h2 = _layernorm(x1) * g2 + sh
            h2_s[r:r + LNR, :] = h2.astype(BF)

    def ffn_up():
        a = jnp.dot(h2_s[...], w1_v[...], preferred_element_type=F32)
        a_s[...] = jnp.maximum(a, 0.0).astype(BF)

    def ffn_down(blk, res_ref, rlo, lo, hi):
        y = jnp.dot(a_s[lo:hi, :], w2_v[...], preferred_element_type=F32)
        r0 = pl.multiple_of(blk * T + lo, 64)
        o_s[pl.ds(r0, hi - lo), :] = (
            res_ref[rlo:rlo + hi - lo, :] + modrow(5) * y).astype(BF)

    @pl.when(pid == 0)
    def _():
        for cpy in (c_copy, x_copy(0), wma_copy, wka_copy, x_copy(1), wkb_copy, wq_copy, wv_copy,
                    wo_copy, wmb_copy, w1_copy, x_copy(2), wmc_copy, w2_copy):
            cpy.start()
        for i in range(3, NBLK):
            x_copy(i).start()
        k_s[0:64, :] = jnp.zeros((64, D), U32)
        c_copy.wait()
        x_copy(0).wait()
        ln1_pre()
        wma_copy.wait()
        mod_part(0, 2 * D)
        ln1(0, hn0_s, hp0_s, True)
        wka_copy.wait()
        k_part(0, hn0_s, 0, HD)
        x_copy(1).wait()
        wkb_copy.wait()
        k_part(0, hn0_s, HD, D)
        ln1(1)
        wq_copy.wait()
        k_part(1)
        wqt_s[...] = wq_v[...].T
        wv_copy.wait()
        q_part(hn0_s)
        wvt_s[...] = wv_v[...].T
        k8_build(0)
        v_part(0, hp0_s)
        v_part(1)
        attention(0, True)
        wo_copy.wait()
        wmb_copy.wait()
        mod_part(2 * D, 5 * D)
        z = attn_proj()
        q_part()
        k8_build(1)
        ln2(0, z)
        wmc_copy.wait()
        w1_copy.wait()
        x_copy(2).wait()
        ln1(2)
        ffn_up()
        mod_part(5 * D, 6 * D)

    @pl.when((pid == 1) | (pid == 2))
    def _():
        @pl.when(pid == 1)
        def _():
            w2_copy.wait()
            x_copy(3).wait()

        @pl.when(pid == 2)
        def _():
            for i in range(4, NBLK):
                x_copy(i).wait()

    @pl.when((pid >= 1) & (pid < NBLK - 1))
    def _():
        attention(pid, False, lambda: ffn_down(pid - 1, x1_s, 0, 0, T))
        z = attn_proj()
        q_part()
        k_part(pid + 1)
        v_part(pid + 1)
        ln2(pid, z)
        ffn_up()
        k8_build(pid + 1)
        ln1(jnp.minimum(pid + 2, NBLK - 1))
        o_copy((pid - 1) * T, T, pid - 1).start()

    @pl.when(pid == NBLK - 1)
    def _():
        last = NBLK - 1
        attention(last, False, lambda: ffn_down(last - 1, x1_s, 0, 0, HT))
        z = attn_proj()
        x1c_s[...] = x1_s[HT:T, :]
        ffn_down(last - 1, x1c_s, 0, HT, T)
        o_copy((last - 1) * T, T, last - 1).start()
        ln2(last, z)
        ffn_up()
        tail = []
        for j, (lo, hi) in enumerate(zip(LASTCUT[:-1], LASTCUT[1:])):
            ffn_down(last, x1_s, lo, lo, hi)
            tail.append(o_copy(last * T + lo, hi - lo, last + j))
            tail[-1].start()
        for i in range(last):
            o_copy(i * T, T, i).wait()
        for cpy in tail:
            cpy.wait()


@jax.jit
def pallas_adaLN_cond__sliding_block__dense_activation_relu__prompt_kernel(
    A_x: jax.Array,
    A_wqkv: jax.Array,
    A_wo: jax.Array,
    B_x: jax.Array,
    B_w1: jax.Array,
    B_w2: jax.Array,
    c: jax.Array,
    w_mod: jax.Array,
):
    del B_x
    x = A_x.reshape(S, D)
    any_spec = pl.BlockSpec(memory_space=pl.ANY)
    scratch = [
        pltpu.VMEM((S, D), BF),
        pltpu.VMEM((D, D), BF),
        pltpu.VMEM((D, D), BF),
        pltpu.VMEM((D, D), BF),
        pltpu.VMEM((D, D), BF),
        pltpu.VMEM((D, DFF), BF),
        pltpu.VMEM((DFF, D), BF),
        pltpu.VMEM((1, D), BF),
        pltpu.VMEM((D, 6 * D), BF),
        pltpu.VMEM((D, D), BF),
        pltpu.VMEM((D, D), BF),
        pltpu.VMEM((8, 6 * D), F32),
        pltpu.VMEM((T, D), BF),
        pltpu.VMEM((HT, D), U32),
        pltpu.VMEM((T, D), BF),
        pltpu.VMEM((HT, D), U32),
        pltpu.VMEM((S // 2 + 64, D), U32),
        pltpu.VMEM((H, S // 2, 128), U32),
        pltpu.VMEM((S // 128, D // 2, 128), U32),
        pltpu.VMEM((D // 2, T), U32),
        pltpu.VMEM((D, T), F32),
        pltpu.VMEM((H, T), F32),
        pltpu.VMEM((T, D), F32),
        pltpu.VMEM((T, D), BF),
        pltpu.VMEM((HT, D), F32),
        pltpu.VMEM((T, DFF), BF),
        pltpu.VMEM((S, D), BF),
        pltpu.SemaphoreType.DMA((NSEM,)),
    ]
    out = pl.pallas_call(
        _kernel,
        grid=(NBLK,),
        in_specs=[any_spec] * 7,
        out_specs=any_spec,
        out_shape=jax.ShapeDtypeStruct((S, D), BF),
        scratch_shapes=scratch,
        compiler_params=pltpu.CompilerParams(
            dimension_semantics=("arbitrary",),
            vmem_limit_bytes=100 * 1024 * 1024),
    )(x, A_wqkv, A_wo, B_w1, B_w2, c, w_mod)
    return out.reshape(1, S, D)
```

```python
import jax
import jax.numpy as jnp
import jax.experimental.pallas as pl
import jax.experimental.pallas.tpu as pltpu

F32 = jnp.float32
BF = jnp.bfloat16
U32 = jnp.uint32

S = 2048
D = 512
H = 32
DFF = 1792
T = 256
HT = T // 2
HD = D // 2
NBLK = S // T
EPS = 1e-5
QSCALE = 0.25 * 1.4426950408889634
NEG = -1e30
NT = (((1,), (1,)), ((), ()))

LNR = 16
L_LO_BITS, L_HI_BITS = (127 - 50) << 23, (127 + 100) << 23
V_LO_BITS, V_HI_BITS = (127 - 40) << 23, (127 + 20) << 23
QK_CUTS = (0, 64, 128, 192, 272)
CUTS0 = (144, 208, 272)
CUTS1 = (16, 80, 144, 208, 272)
DA, DB = 2, 2
DA0, DB0 = 4, 3
LASTCUT = (0, 128, 192, 256)

(SEM_C, SEM_WMA, SEM_WQ, SEM_WV, SEM_WKA, SEM_WKB, SEM_WMB, SEM_WO, SEM_W1, SEM_W2,
 SEM_WMC) = range(11)
SEM_X0 = 11
SEM_O0 = SEM_X0 + NBLK
NSEM = SEM_O0 + NBLK - 1 + len(LASTCUT) - 1


def _u32(x):
    return x if x.dtype == U32 else pltpu.bitcast(x, U32)


def _pack_pairs(a, b):
    return _u32(pltpu.pack_elementwise([a, b], packed_dtype=BF))


def _layernorm(x):
    mu = jnp.mean(x, axis=-1, keepdims=True)
    xc = x - mu
    var = jnp.mean(xc * xc, axis=-1, keepdims=True)
    return xc * jax.lax.rsqrt(var + EPS)


def _kernel(x_hbm, wqkv_hbm, wo_hbm, w1_hbm, w2_hbm, c_hbm, wmod_hbm, out_hbm,
            x_v, wq_v, wk_v, wv_v, wo_v, w1_v, w2_v, c_v, wmod_v,
            wqt_s, wvt_s, mod_s, hn_s, hp_s, hn0_s, hp0_s, k_s, k8_s, vt_s, qt_s, ot_s, l_s,
            x1_s, h2_s, x1c_s, a_s, o_s, hf_s, qf_s, flag_s, vflag_s, sems):
    pid = pl.program_id(0)

    def cp(src, dst, slot):
        return pltpu.make_async_copy(src, dst, sems.at[slot])

    def x_copy(i):
        return cp(x_hbm.at[pl.ds(i * T, T), :], x_v.at[pl.ds(i * T, T), :], SEM_X0 + i)

    def o_copy(r0, n, slot):
        return cp(o_s.at[pl.ds(r0, n), :], out_hbm.at[pl.ds(r0, n), :], SEM_O0 + slot)

    c_copy = cp(c_hbm, c_v, SEM_C)
    wma_copy = cp(wmod_hbm.at[:, pl.ds(0, 2 * D)], wmod_v.at[:, pl.ds(0, 2 * D)], SEM_WMA)
    wmb_copy = cp(wmod_hbm.at[:, pl.ds(2 * D, 3 * D)], wmod_v.at[:, pl.ds(2 * D, 3 * D)], SEM_WMB)
    wmc_copy = cp(wmod_hbm.at[:, pl.ds(5 * D, D)], wmod_v.at[:, pl.ds(5 * D, D)], SEM_WMC)
    wq_copy = cp(wqkv_hbm.at[:, pl.ds(0, D)], wq_v, SEM_WQ)
    wka_copy = cp(wqkv_hbm.at[:, pl.ds(D, HD)], wk_v.at[:, pl.ds(0, HD)], SEM_WKA)
    wkb_copy = cp(wqkv_hbm.at[:, pl.ds(D + HD, HD)], wk_v.at[:, pl.ds(HD, HD)], SEM_WKB)
    wv_copy = cp(wqkv_hbm.at[:, pl.ds(2 * D, D)], wv_v, SEM_WV)
    wo_copy = cp(wo_hbm, wo_v, SEM_WO)
    w1_copy = cp(w1_hbm, w1_v, SEM_W1)
    w2_copy = cp(w2_hbm, w2_v, SEM_W2)

    def mod_part(lo, hi):
        cf = c_v[...].astype(F32)
        sc = cf * (1.0 / (1.0 + jnp.exp(-cf)))
        sc = jnp.broadcast_to(sc, (16, D)).astype(BF)
        m = jnp.dot(sc, wmod_v[:, lo:hi], preferred_element_type=F32)
        mod_s[:, lo:hi] = m[0:8]

    def modrow(k):
        return mod_s[0:1, k * D:(k + 1) * D]

    def ln1_pre():
        for r in range(0, T, LNR):
            x1_s[r:r + LNR, :] = _layernorm(x_v[r:r + LNR, :].astype(F32))

    def ln1(blk, hn_s=hn_s, hp_s=hp_s, pre=False):
        r0 = pl.multiple_of(blk * T, T)
        g1 = 1.0 + modrow(1)
        sh = modrow(0)
        for r in range(0, T, LNR):
            if pre:
                xn = x1_s[r:r + LNR, :]
            else:
                xn = _layernorm(x_v[pl.ds(r0 + r, LNR), :].astype(F32))
            h = xn * g1 + sh
            hn_s[r:r + LNR, :] = h.astype(BF)
            for g in range(LNR // 16):
                hp_s[r // 2 + 8 * g:r // 2 + 8 * g + 8, :] = _pack_pairs(
                    h[16 * g:16 * g + 8], h[16 * g + 8:16 * g + 16])

    def q_part(hn_s=hn_s):
        qt = jax.lax.dot_general(wqt_s[...], hn_s[...], NT, preferred_element_type=F32) * QSCALE
        qt_s[...] = _u32(qt.astype(BF))

    def k_part(blk, hn_s=hn_s, lo=0, hi=D):
        k = jnp.dot(hn_s[...], wk_v[:, lo:hi], preferred_element_type=F32)
        r0 = pl.multiple_of(blk * HT + 64, 64)
        k_s[pl.ds(r0, HT), lo:hi] = _u32(k.astype(BF))

    def v_part(blk, hp_s=hp_s):
        hp = pltpu.bitcast(hp_s[...], BF)
        vt = jax.lax.dot_general(wvt_s[...], hp, NT, preferred_element_type=F32)
        for b in range(T // 128):
            vt_s[blk * (T // 128) + b] = _u32(vt[:, 128 * b:128 * b + 128].astype(BF))

    def fold(x, op):
        t = [x[r:r + 8, c:c + 128] for r in range(0, x.shape[0], 8)
             for c in range(0, x.shape[1], 128)]
        while len(t) > 1:
            t = [op(t[i], t[i + 1]) for i in range(0, len(t), 2)]
        return t[0]

    def v_check(blk):
        mn = mx = None
        for b in range(T // 128):
            for r in range(0, D // 2, 8):
                u = pltpu.bitcast(vt_s[blk * (T // 128) + b, r:r + 8, :], jnp.int32)
                for m in (u & 0x7FFF0000, (u << 16) & 0x7FFF0000):
                    nz = (m - 0x10000) & 0x7FFF0000
                    mn = nz if mn is None else jnp.minimum(mn, nz)
                    mx = m if mx is None else jnp.maximum(mx, m)
        bad = (mn < V_LO_BITS) | (mx > V_HI_BITS)
        vflag_s[blk] = jnp.where(bad, 1, 0)

    def k8_build(blk):
        lane = jax.lax.broadcasted_iota(jnp.int32, (8, 128), 1)
        bit = [((lane >> (4 + k)) & 1) == 1 for k in range(3)]
        src0 = blk * HT + 8
        dst0 = blk * HT
        for g in range(4):
            xs = {}

            def x(w, g=g, xs=xs):
                if w not in xs:
                    xs[w] = k_s[pl.ds(pl.multiple_of(src0 + 8 * w, 8), 8), 128 * g:128 * g + 128]
                return xs[w]

            for u in range(T // 16):
                f = [x(u)] + [pltpu.roll(x(u + d), 16 * d, 1) for d in range(1, 8)]
                for k in range(3):
                    f = [jnp.where(bit[k], f[(m + (1 << k)) % 8], f[m]) for m in range(8)]
                for hh in range(8):
                    k8_s[8 * g + hh, pl.ds(pl.multiple_of(dst0 + 8 * u, 8), 8), :] = f[(-hh) % 8]

    def attention(blk, first, filler=None, safe=False):
        lane8 = jax.lax.broadcasted_iota(jnp.int32, (8, 128), 1)
        srow = jax.lax.broadcasted_iota(jnp.int32, (8, 128), 0)
        i16 = lane8 & 15
        first_m = [8 * v + srow > i16 for v in range(2)]
        last_m = [8 * v + srow <= i16 for v in range(2)]
        blkid = lane8 >> 4
        blkge = [blkid >= s for s in range(8)]
        bit = [((blkid >> k) & 1) == 1 for k in range(3)]
        zero8 = jnp.zeros((8, 128), U32)
        neg8 = jnp.full((8, 128), NEG, F32)

        def rows(h, n):
            return pl.ds(pl.multiple_of(n * h, n), n)

        def qk(b, h):
            nneg = max(0, 256 - 128 * b) if first else 0
            tmin = max(0, nneg - 112)
            cuts = QK_CUTS if tmin == 0 else (CUTS1 if tmin == 16 else CUTS0)
            if safe:
                qv = qf_s[rows(h, 8), 128 * b:128 * b + 128]
                parts = [jnp.where(blkid == ((s - h) & 7), qv, zero8) for s in range(8)]
                cuts = (cuts[0], cuts[-1])
            else:
                lvl = [qt_s[8 * h:8 * h + 8, 128 * b:128 * b + 128]]
                for k in (2, 1, 0):
                    lvl = [x for y in lvl
                           for x in (jnp.where(bit[k], zero8, y), jnp.where(bit[k], y, zero8))]
                parts = [lvl[(s - h) % 8] for s in range(8)]
            w = pltpu.bitcast(jnp.concatenate(parts, axis=0), BF)
            sv = {}
            row0 = blk * HT + 64 * b - 72
            for a_, b_ in zip(cuts[:-1], cuts[1:]):
                kc = k8_s[h, pl.ds(pl.multiple_of(row0 + a_ // 2, 8), (b_ - a_) // 2), :]
                sc = jnp.dot(pltpu.bitcast(kc, BF), w, preferred_element_type=F32)
                for v in range((b_ - a_) // 8):
                    sv[a_ // 8 + v] = sc[8 * v:8 * v + 8]
            return sv, nneg

        def mask_max(sv, nneg):
            for v in sorted(sv):
                if v < 2:
                    sv[v] = jnp.where(first_m[v], sv[v], neg8)
                elif v >= 32:
                    sv[v] = jnp.where(last_m[v - 32], sv[v], neg8)
                if 8 * v < nneg:
                    smin = -((8 * v - nneg) // 16)
                    sv[v] = jnp.where(blkge[smin], sv[v], neg8)
            if not safe:
                return None, sv
            vs = sorted(sv)
            m0, m1 = sv[vs[0]], sv[vs[1]]
            for v in vs[2::2]:
                m0 = jnp.maximum(m0, sv[v])
                m1 = jnp.maximum(m1, sv[v + 1])
            m = jnp.max(jnp.maximum(m0, m1), axis=0, keepdims=True)
            return jnp.broadcast_to(m, (8, 128)), sv

        def probs(b, h, st):
            m, sv = st
            c0 = max(0, 2 - b) if first else 0
            lv = [{}, {}, {}]
            outv = []

            def sel(mk, a, c):
                if a is None and c is None:
                    return None
                return jnp.where(mk, zero8 if a is None else a, zero8 if c is None else c)

            l0 = l1 = None
            for v in range(24):
                if v < 17 and 2 * v in sv:
                    a = jnp.exp2(sv[2 * v] - m if safe else sv[2 * v])
                    c = jnp.exp2(sv[2 * v + 1] - m if safe else sv[2 * v + 1])
                    l0 = a if l0 is None else l0 + a
                    l1 = c if l1 is None else l1 + c
                    lv[0][v] = _pack_pairs(a, c)
                if v < 18:
                    lv[1][v] = sel(bit[0], lv[0].get(v - 1), lv[0].get(v))
                if v < 20:
                    lv[2][v] = sel(bit[1], lv[1].get(v - 2), lv[1].get(v))
                if v >= 8 * c0:
                    o = sel(bit[2], lv[2].get(v - 4), lv[2].get(v))
                    outv.append(zero8 if o is None else o)
            l = jnp.sum(l0 + l1, axis=0, keepdims=True)
            if safe:
                return outv, l
            l_s[h:h + 1, 128 * b:128 * b + 128] = l
            return outv, None

        def pv(b, h, st):
            outv, l = st
            c0 = max(0, 2 - b) if first else 0
            tile0 = blk * (T // 128) + b - 2
            acc = None
            for c in range(c0, 3):
                pt = pltpu.bitcast(
                    jnp.concatenate(outv[8 * (c - c0):8 * (c - c0) + 8], axis=0), BF)
                vt = vt_s[tile0 + c, rows(h, 8), :]
                o = jnp.dot(pltpu.bitcast(vt, BF), pt, preferred_element_type=F32)
                acc = o if acc is None else acc + o
            if safe:
                acc = acc * (1.0 / l)
            ot_s[rows(h, 16), 128 * b:128 * b + 128] = acc

        if safe:
            for b in range(T // 128):
                def head(h, carry, b=b):
                    pv(b, h, probs(b, h, mask_max(*qk(b, h))))
                    return carry

                jax.lax.fori_loop(0, H, head, 0)
            return

        items = [(b, h) for b in range(T // 128) for h in range(H)]
        n = len(items)
        sa, sb = {}, {}
        da, db = (DA0, DB0) if first else (DA, DB)
        for t in range(n + da + db):
            st = qk(*items[t]) if t < n else None
            if 0 <= t - da < n:
                sb[t - da] = probs(*items[t - da], sa.pop(t - da))
            if 0 <= t - da - db < n:
                pv(*items[t - da - db], sb.pop(t - da - db))
            if st is not None:
                sa[t] = mask_max(*st)
            if filler is not None and t == n:
                filler()

    def attn_proj(blk):
        l = l_s[...]
        rl = 1.0 / l
        parts = [ot_s[16 * h:16 * h + 16, :] * rl[h:h + 1, :] for h in range(H)]
        li = pltpu.bitcast(l, jnp.int32)
        bad = (fold(li, jnp.minimum) < L_LO_BITS) | (fold(li, jnp.maximum) > L_HI_BITS)
        flag_s[blk] = jnp.where(bad, 1, 0)
        o = jnp.concatenate(parts, axis=0).T.astype(BF)
        return jnp.dot(o, wo_v[...], preferred_element_type=F32)

    def ln2(blk, z):
        r0 = pl.multiple_of(blk * T, T)
        g2 = 1.0 + modrow(4)
        sh = modrow(3)
        ga = modrow(2)
        for r in range(0, T, LNR):
            x1 = x_v[pl.ds(r0 + r, LNR), :].astype(F32) + ga * z[r:r + LNR]
            x1_s[r:r + LNR, :] = x1
            h2 = _layernorm(x1) * g2 + sh
            h2_s[r:r + LNR, :] = h2.astype(BF)

    def ffn_up():
        a = jnp.dot(h2_s[...], w1_v[...], preferred_element_type=F32)
        a_s[...] = jnp.maximum(a, 0.0).astype(BF)

    def ffn_down(blk, res_ref, rlo, lo, hi):
        y = jnp.dot(a_s[lo:hi, :], w2_v[...], preferred_element_type=F32)
        r0 = pl.multiple_of(blk * T + lo, 64)
        o_s[pl.ds(r0, hi - lo), :] = (
            res_ref[rlo:rlo + hi - lo, :] + modrow(5) * y).astype(BF)

    def redo(blk, first):
        r0 = pl.multiple_of(blk * T, T)
        g1 = 1.0 + modrow(1)
        sh1 = modrow(0)

        def ln_rows(i, carry):
            r = pl.multiple_of(i * 16, 16)
            xn = _layernorm(x_v[pl.ds(pl.multiple_of(r0 + r, 16), 16), :].astype(F32))
            hf_s[pl.ds(r, 16), :] = (xn * g1 + sh1).astype(BF)
            return carry

        jax.lax.fori_loop(0, T // 16, ln_rows, 0)

        def q_rows(j, carry):
            wt = wqt_s[pl.ds(pl.multiple_of(j * 128, 128), 128), :]
            qt = jax.lax.dot_general(wt, hf_s[...], NT, preferred_element_type=F32) * QSCALE
            qf_s[pl.ds(pl.multiple_of(j * 64, 64), 64), :] = _u32(qt.astype(BF))
            return carry

        jax.lax.fori_loop(0, D // 128, q_rows, 0)
        attention(blk, first, safe=True)
        hf_s[...] = ot_s[...].T.astype(BF)
        g2 = 1.0 + modrow(4)
        sh2 = modrow(3)
        ga = modrow(2)
        gb = modrow(5)

        def tail_rows(i, carry):
            r = pl.multiple_of(i * 32, 32)
            rows = pl.ds(pl.multiple_of(r0 + r, 32), 32)
            z = jnp.dot(hf_s[pl.ds(r, 32), :], wo_v[...], preferred_element_type=F32)
            x1 = x_v[rows, :].astype(F32) + ga * z
            h2 = (_layernorm(x1) * g2 + sh2).astype(BF)
            a = jnp.dot(h2, w1_v[...], preferred_element_type=F32)
            a = jnp.maximum(a, 0.0).astype(BF)
            y = jnp.dot(a, w2_v[...], preferred_element_type=F32)
            o_s[rows, :] = (x1 + gb * y).astype(BF)
            return carry

        jax.lax.fori_loop(0, T // 32, tail_rows, 0)
        cpy = o_copy(r0, T, 0)
        cpy.start()
        cpy.wait()

    @pl.when(pid == 0)
    def _():
        for cpy in (c_copy, x_copy(0), wma_copy, wka_copy, x_copy(1), wkb_copy, wq_copy, wv_copy,
                    wo_copy, wmb_copy, w1_copy, x_copy(2), wmc_copy, w2_copy):
            cpy.start()
        for i in range(3, NBLK):
            x_copy(i).start()
        k_s[0:64, :] = jnp.zeros((64, D), U32)
        c_copy.wait()
        x_copy(0).wait()
        ln1_pre()
        wma_copy.wait()
        mod_part(0, 2 * D)
        ln1(0, hn0_s, hp0_s, True)
        wka_copy.wait()
        k_part(0, hn0_s, 0, HD)
        x_copy(1).wait()
        wkb_copy.wait()
        k_part(0, hn0_s, HD, D)
        ln1(1)
        wq_copy.wait()
        k_part(1)
        wqt_s[...] = wq_v[...].T
        wv_copy.wait()
        q_part(hn0_s)
        wvt_s[...] = wv_v[...].T
        k8_build(0)
        v_part(0, hp0_s)
        v_part(1)
        v_check(0)
        v_check(1)
        attention(0, True)
        wo_copy.wait()
        wmb_copy.wait()
        mod_part(2 * D, 5 * D)
        z = attn_proj(0)
        q_part()
        k8_build(1)
        ln2(0, z)
        wmc_copy.wait()
        w1_copy.wait()
        x_copy(2).wait()
        ln1(2)
        ffn_up()
        mod_part(5 * D, 6 * D)

    @pl.when((pid == 1) | (pid == 2))
    def _():
        @pl.when(pid == 1)
        def _():
            w2_copy.wait()
            x_copy(3).wait()

        @pl.when(pid == 2)
        def _():
            for i in range(4, NBLK):
                x_copy(i).wait()

    @pl.when((pid >= 1) & (pid < NBLK - 1))
    def _():
        attention(pid, False, lambda: ffn_down(pid - 1, x1_s, 0, 0, T))
        z = attn_proj(pid)
        q_part()
        k_part(pid + 1)
        v_part(pid + 1)
        ln2(pid, z)
        ffn_up()
        k8_build(pid + 1)
        v_check(pid + 1)
        ln1(jnp.minimum(pid + 2, NBLK - 1))
        o_copy((pid - 1) * T, T, pid - 1).start()

    @pl.when(pid == NBLK - 1)
    def _():
        last = NBLK - 1
        attention(last, False, lambda: ffn_down(last - 1, x1_s, 0, 0, HT))
        z = attn_proj(last)
        x1c_s[...] = x1_s[HT:T, :]
        ffn_down(last - 1, x1c_s, 0, HT, T)
        o_copy((last - 1) * T, T, last - 1).start()
        ln2(last, z)
        ffn_up()
        tail = []
        for j, (lo, hi) in enumerate(zip(LASTCUT[:-1], LASTCUT[1:])):
            ffn_down(last, x1_s, lo, lo, hi)
            tail.append(o_copy(last * T + lo, hi - lo, last + j))
            tail[-1].start()
        v_bad = fold(vflag_s[...].reshape(NBLK * 8, 128), jnp.maximum)
        any_bad = jnp.max(
            jnp.maximum(fold(flag_s[...].reshape(NBLK * 8, 128), jnp.maximum), v_bad))
        for i in range(last):
            o_copy(i * T, T, i).wait()
        for cpy in tail:
            cpy.wait()

        @pl.when(any_bad > 0)
        def _():
            @pl.when(jnp.max(jnp.maximum(flag_s[0], v_bad)) > 0)
            def _():
                redo(0, True)

            def one(blk, carry):
                @pl.when(jnp.max(jnp.maximum(flag_s[blk], v_bad)) > 0)
                def _():
                    redo(blk, False)

                return carry

            jax.lax.fori_loop(1, NBLK, one, 0)


@jax.jit
def pallas_adaLN_cond__sliding_block__dense_activation_relu__prompt_kernel(
    A_x: jax.Array,
    A_wqkv: jax.Array,
    A_wo: jax.Array,
    B_x: jax.Array,
    B_w1: jax.Array,
    B_w2: jax.Array,
    c: jax.Array,
    w_mod: jax.Array,
):
    del B_x
    x = A_x.reshape(S, D)
    any_spec = pl.BlockSpec(memory_space=pl.ANY)
    scratch = [
        pltpu.VMEM((S, D), BF),
        pltpu.VMEM((D, D), BF),
        pltpu.VMEM((D, D), BF),
        pltpu.VMEM((D, D), BF),
        pltpu.VMEM((D, D), BF),
        pltpu.VMEM((D, DFF), BF),
        pltpu.VMEM((DFF, D), BF),
        pltpu.VMEM((1, D), BF),
        pltpu.VMEM((D, 6 * D), BF),
        pltpu.VMEM((D, D), BF),
        pltpu.VMEM((D, D), BF),
        pltpu.VMEM((8, 6 * D), F32),
        pltpu.VMEM((T, D), BF),
        pltpu.VMEM((HT, D), U32),
        pltpu.VMEM((T, D), BF),
        pltpu.VMEM((HT, D), U32),
        pltpu.VMEM((S // 2 + 64, D), U32),
        pltpu.VMEM((H, S // 2, 128), U32),
        pltpu.VMEM((S // 128, D // 2, 128), U32),
        pltpu.VMEM((D // 2, T), U32),
        pltpu.VMEM((D, T), F32),
        pltpu.VMEM((H, T), F32),
        pltpu.VMEM((T, D), F32),
        pltpu.VMEM((T, D), BF),
        pltpu.VMEM((HT, D), F32),
        pltpu.VMEM((T, DFF), BF),
        pltpu.VMEM((S, D), BF),
        pltpu.VMEM((T, D), BF),
        pltpu.VMEM((D // 2, T), U32),
        pltpu.VMEM((NBLK, 8, 128), jnp.int32),
        pltpu.VMEM((NBLK, 8, 128), jnp.int32),
        pltpu.SemaphoreType.DMA((NSEM,)),
    ]
    out = pl.pallas_call(
        _kernel,
        grid=(NBLK,),
        in_specs=[any_spec] * 7,
        out_specs=any_spec,
        out_shape=jax.ShapeDtypeStruct((S, D), BF),
        scratch_shapes=scratch,
        compiler_params=pltpu.CompilerParams(
            dimension_semantics=("arbitrary",),
            vmem_limit_bytes=100 * 1024 * 1024),
    )(x, A_wqkv, A_wo, B_w1, B_w2, c, w_mod)
    return out.reshape(1, S, D)
```

```python
import jax
import jax.numpy as jnp
import jax.experimental.pallas as pl
import jax.experimental.pallas.tpu as pltpu

F32 = jnp.float32
BF = jnp.bfloat16
U32 = jnp.uint32

S = 2048
D = 512
H = 32
DFF = 1792
T = 256
HT = T // 2
HD = D // 2
NBLK = S // T
EPS = 1e-5
QSCALE = 0.25 * 1.4426950408889634
NEG = -1e30
NT = (((1,), (1,)), ((), ()))

LNR = 16
L_LO_BITS, L_HI_BITS = (127 - 50) << 23, (127 + 100) << 23
V_LO_BITS, V_HI_BITS = (127 - 40) << 23, (127 + 20) << 23
QK_CUTS = (0, 64, 128, 192, 272)
CUTS0 = (144, 208, 272)
CUTS1 = (16, 80, 144, 208, 272)
DA = 2
DB = 1
DA0 = 5
DB0 = 3
LASTCUT = (0, 128, 192, 256)

(SEM_C, SEM_WMA, SEM_WQ, SEM_WV, SEM_WKA, SEM_WKB, SEM_WMB, SEM_WO, SEM_W1, SEM_W2,
 SEM_WMC) = range(11)
SEM_X0 = 11
SEM_O0 = SEM_X0 + NBLK
NSEM = SEM_O0 + NBLK - 1 + len(LASTCUT) - 1


def _u32(x):
    return x if x.dtype == U32 else pltpu.bitcast(x, U32)


def _pack_pairs(a, b):
    return _u32(pltpu.pack_elementwise([a, b], packed_dtype=BF))


def _layernorm(x):
    mu = jnp.mean(x, axis=-1, keepdims=True)
    xc = x - mu
    var = jnp.mean(xc * xc, axis=-1, keepdims=True)
    return xc * jax.lax.rsqrt(var + EPS)


def _kernel(x_hbm, wqkv_hbm, wo_hbm, w1_hbm, w2_hbm, c_hbm, wmod_hbm, out_hbm,
            x_v, wq_v, wk_v, wv_v, wo_v, w1_v, w2_v, c_v, wmod_v,
            wqt_s, wvt_s, mod_s, hn_s, hp_s, hn0_s, hp0_s, k_s, k8_s, vt_s, qt_s, ot_s, l_s,
            x1_s, h2_s, x1c_s, a_s, o_s, hf_s, qf_s, flag_s, vflag_s, sems):
    pid = pl.program_id(0)

    def cp(src, dst, slot):
        return pltpu.make_async_copy(src, dst, sems.at[slot])

    def x_copy(i):
        return cp(x_hbm.at[pl.ds(i * T, T), :], x_v.at[pl.ds(i * T, T), :], SEM_X0 + i)

    def o_copy(r0, n, slot):
        return cp(o_s.at[pl.ds(r0, n), :], out_hbm.at[pl.ds(r0, n), :], SEM_O0 + slot)

    c_copy = cp(c_hbm, c_v, SEM_C)
    wma_copy = cp(wmod_hbm.at[:, pl.ds(0, 2 * D)], wmod_v.at[:, pl.ds(0, 2 * D)], SEM_WMA)
    wmb_copy = cp(wmod_hbm.at[:, pl.ds(2 * D, 3 * D)], wmod_v.at[:, pl.ds(2 * D, 3 * D)], SEM_WMB)
    wmc_copy = cp(wmod_hbm.at[:, pl.ds(5 * D, D)], wmod_v.at[:, pl.ds(5 * D, D)], SEM_WMC)
    wq_copy = cp(wqkv_hbm.at[:, pl.ds(0, D)], wq_v, SEM_WQ)
    wka_copy = cp(wqkv_hbm.at[:, pl.ds(D, HD)], wk_v.at[:, pl.ds(0, HD)], SEM_WKA)
    wkb_copy = cp(wqkv_hbm.at[:, pl.ds(D + HD, HD)], wk_v.at[:, pl.ds(HD, HD)], SEM_WKB)
    wv_copy = cp(wqkv_hbm.at[:, pl.ds(2 * D, D)], wv_v, SEM_WV)
    wo_copy = cp(wo_hbm, wo_v, SEM_WO)
    w1_copy = cp(w1_hbm, w1_v, SEM_W1)
    w2_copy = cp(w2_hbm, w2_v, SEM_W2)

    def mod_part(lo, hi):
        cf = c_v[...].astype(F32)
        sc = cf * (1.0 / (1.0 + jnp.exp(-cf)))
        sc = jnp.broadcast_to(sc, (16, D)).astype(BF)
        m = jnp.dot(sc, wmod_v[:, lo:hi], preferred_element_type=F32)
        mod_s[:, lo:hi] = m[0:8]

    def modrow(k):
        return mod_s[0:1, k * D:(k + 1) * D]

    def ln1_pre():
        for r in range(0, T, LNR):
            x1_s[r:r + LNR, :] = _layernorm(x_v[r:r + LNR, :].astype(F32))

    def ln1(blk, hn_s=hn_s, hp_s=hp_s, pre=False):
        r0 = pl.multiple_of(blk * T, T)
        g1 = 1.0 + modrow(1)
        sh = modrow(0)
        for r in range(0, T, LNR):
            if pre:
                xn = x1_s[r:r + LNR, :]
            else:
                xn = _layernorm(x_v[pl.ds(r0 + r, LNR), :].astype(F32))
            h = xn * g1 + sh
            hn_s[r:r + LNR, :] = h.astype(BF)
            for g in range(LNR // 16):
                hp_s[r // 2 + 8 * g:r // 2 + 8 * g + 8, :] = _pack_pairs(
                    h[16 * g:16 * g + 8], h[16 * g + 8:16 * g + 16])

    def q_part(hn_s=hn_s):
        qt = jax.lax.dot_general(wqt_s[...], hn_s[...], NT, preferred_element_type=F32) * QSCALE
        qt_s[...] = _u32(qt.astype(BF))

    def k_part(blk, hn_s=hn_s, lo=0, hi=D):
        k = jnp.dot(hn_s[...], wk_v[:, lo:hi], preferred_element_type=F32)
        r0 = pl.multiple_of(blk * HT + 64, 64)
        k_s[pl.ds(r0, HT), lo:hi] = _u32(k.astype(BF))

    def v_part(blk, hp_s=hp_s):
        hp = pltpu.bitcast(hp_s[...], BF)
        vt = jax.lax.dot_general(wvt_s[...], hp, NT, preferred_element_type=F32)
        for b in range(T // 128):
            vt_s[blk * (T // 128) + b] = _u32(vt[:, 128 * b:128 * b + 128].astype(BF))

    def fold(x, op):
        t = [x[r:r + 8, c:c + 128] for r in range(0, x.shape[0], 8)
             for c in range(0, x.shape[1], 128)]
        while len(t) > 1:
            t = [op(t[i], t[i + 1]) for i in range(0, len(t), 2)]
        return t[0]

    def v_check(blk):
        mn = mx = None
        for b in range(T // 128):
            for r in range(0, D // 2, 8):
                u = pltpu.bitcast(vt_s[blk * (T // 128) + b, r:r + 8, :], jnp.int32)
                for m in (u & 0x7FFF0000, (u << 16) & 0x7FFF0000):
                    nz = (m - 0x10000) & 0x7FFF0000
                    mn = nz if mn is None else jnp.minimum(mn, nz)
                    mx = m if mx is None else jnp.maximum(mx, m)
        bad = (mn < V_LO_BITS) | (mx > V_HI_BITS)
        vflag_s[blk] = jnp.where(bad, 1, 0)

    def k8_build(blk):
        lane = jax.lax.broadcasted_iota(jnp.int32, (8, 128), 1)
        bit = [((lane >> (4 + k)) & 1) == 1 for k in range(3)]
        src0 = blk * HT + 8
        dst0 = blk * HT
        for g in range(4):
            xs = {}

            def x(w, g=g, xs=xs):
                if w not in xs:
                    xs[w] = k_s[pl.ds(pl.multiple_of(src0 + 8 * w, 8), 8), 128 * g:128 * g + 128]
                return xs[w]

            for u in range(T // 16):
                f = [x(u)] + [pltpu.roll(x(u + d), 16 * d, 1) for d in range(1, 8)]
                for k in range(3):
                    f = [jnp.where(bit[k], f[(m + (1 << k)) % 8], f[m]) for m in range(8)]
                for hh in range(8):
                    k8_s[8 * g + hh, pl.ds(pl.multiple_of(dst0 + 8 * u, 8), 8), :] = f[(-hh) % 8]

    def attention(blk, first, filler=None, safe=False):
        lane8 = jax.lax.broadcasted_iota(jnp.int32, (8, 128), 1)
        srow = jax.lax.broadcasted_iota(jnp.int32, (8, 128), 0)
        i16 = lane8 & 15
        first_m = [8 * v + srow > i16 for v in range(2)]
        last_m = [8 * v + srow <= i16 for v in range(2)]
        blkid = lane8 >> 4
        blkge = [blkid >= s for s in range(8)]
        bit = [((blkid >> k) & 1) == 1 for k in range(3)]
        zero8 = jnp.zeros((8, 128), U32)
        neg8 = jnp.full((8, 128), NEG, F32)

        def rows(h, n):
            return pl.ds(pl.multiple_of(n * h, n), n)

        def qk(b, h):
            nneg = max(0, 256 - 128 * b) if first else 0
            tmin = max(0, nneg - 112)
            cuts = QK_CUTS if tmin == 0 else (CUTS1 if tmin == 16 else CUTS0)
            if safe:
                qv = qf_s[rows(h, 8), 128 * b:128 * b + 128]
                parts = [jnp.where(blkid == ((s - h) & 7), qv, zero8) for s in range(8)]
                cuts = (cuts[0], cuts[-1])
            else:
                lvl = [qt_s[8 * h:8 * h + 8, 128 * b:128 * b + 128]]
                for k in (2, 1, 0):
                    lvl = [x for y in lvl
                           for x in (jnp.where(bit[k], zero8, y), jnp.where(bit[k], y, zero8))]
                parts = [lvl[(s - h) % 8] for s in range(8)]
            w = pltpu.bitcast(jnp.concatenate(parts, axis=0), BF)
            sv = {}
            row0 = blk * HT + 64 * b - 72
            for a_, b_ in zip(cuts[:-1], cuts[1:]):
                kc = k8_s[h, pl.ds(pl.multiple_of(row0 + a_ // 2, 8), (b_ - a_) // 2), :]
                sc = jnp.dot(pltpu.bitcast(kc, BF), w, preferred_element_type=F32)
                for v in range((b_ - a_) // 8):
                    sv[a_ // 8 + v] = sc[8 * v:8 * v + 8]
            return sv, nneg

        def mask_max(sv, nneg):
            for v in sorted(sv):
                if v < 2:
                    sv[v] = jnp.where(first_m[v], sv[v], neg8)
                elif v >= 32:
                    sv[v] = jnp.where(last_m[v - 32], sv[v], neg8)
                if 8 * v < nneg:
                    smin = -((8 * v - nneg) // 16)
                    sv[v] = jnp.where(blkge[smin], sv[v], neg8)
            if not safe:
                return None, sv
            vs = sorted(sv)
            m0, m1 = sv[vs[0]], sv[vs[1]]
            for v in vs[2::2]:
                m0 = jnp.maximum(m0, sv[v])
                m1 = jnp.maximum(m1, sv[v + 1])
            m = jnp.max(jnp.maximum(m0, m1), axis=0, keepdims=True)
            return jnp.broadcast_to(m, (8, 128)), sv

        def probs(b, h, st):
            m, sv = st
            c0 = max(0, 2 - b) if first else 0
            lv = [{}, {}, {}]
            outv = []

            def sel(mk, a, c):
                if a is None and c is None:
                    return None
                return jnp.where(mk, zero8 if a is None else a, zero8 if c is None else c)

            l0 = l1 = None
            for v in range(24):
                if v < 17 and 2 * v in sv:
                    a = jnp.exp2(sv[2 * v] - m if safe else sv[2 * v])
                    c = jnp.exp2(sv[2 * v + 1] - m if safe else sv[2 * v + 1])
                    l0 = a if l0 is None else l0 + a
                    l1 = c if l1 is None else l1 + c
                    lv[0][v] = _pack_pairs(a, c)
                if v < 18:
                    lv[1][v] = sel(bit[0], lv[0].get(v - 1), lv[0].get(v))
                if v < 20:
                    lv[2][v] = sel(bit[1], lv[1].get(v - 2), lv[1].get(v))
                if v >= 8 * c0:
                    o = sel(bit[2], lv[2].get(v - 4), lv[2].get(v))
                    outv.append(zero8 if o is None else o)
            l = jnp.sum(l0 + l1, axis=0, keepdims=True)
            if safe:
                return outv, l
            l_s[h:h + 1, 128 * b:128 * b + 128] = l
            return outv, None

        def pv(b, h, st):
            outv, l = st
            c0 = max(0, 2 - b) if first else 0
            tile0 = blk * (T // 128) + b - 2
            acc = None
            for c in range(c0, 3):
                pt = pltpu.bitcast(
                    jnp.concatenate(outv[8 * (c - c0):8 * (c - c0) + 8], axis=0), BF)
                vt = vt_s[tile0 + c, rows(h, 8), :]
                o = jnp.dot(pltpu.bitcast(vt, BF), pt, preferred_element_type=F32)
                acc = o if acc is None else acc + o
            if safe:
                acc = acc * (1.0 / l)
            ot_s[rows(h, 16), 128 * b:128 * b + 128] = acc

        if safe:
            for b in range(T // 128):
                def head(h, carry, b=b):
                    pv(b, h, probs(b, h, mask_max(*qk(b, h))))
                    return carry

                jax.lax.fori_loop(0, H, head, 0)
            return

        items = [(b, h) for b in range(T // 128) for h in range(H)]
        n = len(items)
        sa, sb = {}, {}
        da, db = (DA0, DB0) if first else (DA, DB)
        for t in range(n + da + db):
            st = qk(*items[t]) if t < n else None
            if 0 <= t - da < n:
                sb[t - da] = probs(*items[t - da], sa.pop(t - da))
            if 0 <= t - da - db < n:
                pv(*items[t - da - db], sb.pop(t - da - db))
            if st is not None:
                sa[t] = mask_max(*st)
            if filler is not None and t == n:
                filler()

    def attn_proj(blk):
        l = l_s[...]
        rl = 1.0 / l
        parts = [ot_s[16 * h:16 * h + 16, :] * rl[h:h + 1, :] for h in range(H)]
        li = pltpu.bitcast(l, jnp.int32)
        bad = (fold(li, jnp.minimum) < L_LO_BITS) | (fold(li, jnp.maximum) > L_HI_BITS)
        flag_s[blk] = jnp.where(bad, 1, 0)
        o = jnp.concatenate(parts, axis=0).T.astype(BF)
        return jnp.dot(o, wo_v[...], preferred_element_type=F32)

    def ln2(blk, z):
        r0 = pl.multiple_of(blk * T, T)
        g2 = 1.0 + modrow(4)
        sh = modrow(3)
        ga = modrow(2)
        for r in range(0, T, LNR):
            x1 = x_v[pl.ds(r0 + r, LNR), :].astype(F32) + ga * z[r:r + LNR]
            x1_s[r:r + LNR, :] = x1
            h2 = _layernorm(x1) * g2 + sh
            h2_s[r:r + LNR, :] = h2.astype(BF)

    def ffn_up():
        a = jnp.dot(h2_s[...], w1_v[...], preferred_element_type=F32)
        a_s[...] = jnp.maximum(a, 0.0).astype(BF)

    def ffn_down(blk, res_ref, rlo, lo, hi):
        y = jnp.dot(a_s[lo:hi, :], w2_v[...], preferred_element_type=F32)
        r0 = pl.multiple_of(blk * T + lo, 64)
        o_s[pl.ds(r0, hi - lo), :] = (
            res_ref[rlo:rlo + hi - lo, :] + modrow(5) * y).astype(BF)

    def redo(blk, first):
        r0 = pl.multiple_of(blk * T, T)
        g1 = 1.0 + modrow(1)
        sh1 = modrow(0)

        def ln_rows(i, carry):
            r = pl.multiple_of(i * 16, 16)
            xn = _layernorm(x_v[pl.ds(pl.multiple_of(r0 + r, 16), 16), :].astype(F32))
            hf_s[pl.ds(r, 16), :] = (xn * g1 + sh1).astype(BF)
            return carry

        jax.lax.fori_loop(0, T // 16, ln_rows, 0)

        def q_rows(j, carry):
            wt = wqt_s[pl.ds(pl.multiple_of(j * 128, 128), 128), :]
            qt = jax.lax.dot_general(wt, hf_s[...], NT, preferred_element_type=F32) * QSCALE
            qf_s[pl.ds(pl.multiple_of(j * 64, 64), 64), :] = _u32(qt.astype(BF))
            return carry

        jax.lax.fori_loop(0, D // 128, q_rows, 0)
        attention(blk, first, safe=True)
        hf_s[...] = ot_s[...].T.astype(BF)
        g2 = 1.0 + modrow(4)
        sh2 = modrow(3)
        ga = modrow(2)
        gb = modrow(5)

        def tail_rows(i, carry):
            r = pl.multiple_of(i * 32, 32)
            rows = pl.ds(pl.multiple_of(r0 + r, 32), 32)
            z = jnp.dot(hf_s[pl.ds(r, 32), :], wo_v[...], preferred_element_type=F32)
            x1 = x_v[rows, :].astype(F32) + ga * z
            h2 = (_layernorm(x1) * g2 + sh2).astype(BF)
            a = jnp.dot(h2, w1_v[...], preferred_element_type=F32)
            a = jnp.maximum(a, 0.0).astype(BF)
            y = jnp.dot(a, w2_v[...], preferred_element_type=F32)
            o_s[rows, :] = (x1 + gb * y).astype(BF)
            return carry

        jax.lax.fori_loop(0, T // 32, tail_rows, 0)
        cpy = o_copy(r0, T, 0)
        cpy.start()
        cpy.wait()

    @pl.when(pid == 0)
    def _():
        for cpy in (c_copy, x_copy(0), wma_copy, wka_copy, x_copy(1), wkb_copy, wq_copy, wv_copy,
                    wo_copy, wmb_copy, w1_copy, x_copy(2), wmc_copy, w2_copy):
            cpy.start()
        for i in range(3, NBLK):
            x_copy(i).start()
        k_s[0:64, :] = jnp.zeros((64, D), U32)
        c_copy.wait()
        x_copy(0).wait()
        ln1_pre()
        wma_copy.wait()
        mod_part(0, 2 * D)
        ln1(0, hn0_s, hp0_s, True)
        wka_copy.wait()
        k_part(0, hn0_s, 0, HD)
        x_copy(1).wait()
        wkb_copy.wait()
        k_part(0, hn0_s, HD, D)
        ln1(1)
        wq_copy.wait()
        k_part(1)
        wqt_s[...] = wq_v[...].T
        wv_copy.wait()
        q_part(hn0_s)
        wvt_s[...] = wv_v[...].T
        k8_build(0)
        v_part(0, hp0_s)
        v_part(1)
        v_check(0)
        v_check(1)
        attention(0, True)
        wo_copy.wait()
        wmb_copy.wait()
        mod_part(2 * D, 5 * D)
        z = attn_proj(0)
        q_part()
        k8_build(1)
        ln2(0, z)
        wmc_copy.wait()
        w1_copy.wait()
        x_copy(2).wait()
        ln1(2)
        ffn_up()
        mod_part(5 * D, 6 * D)

    @pl.when((pid == 1) | (pid == 2))
    def _():
        @pl.when(pid == 1)
        def _():
            w2_copy.wait()
            x_copy(3).wait()

        @pl.when(pid == 2)
        def _():
            for i in range(4, NBLK):
                x_copy(i).wait()

    @pl.when((pid >= 1) & (pid < NBLK - 1))
    def _():
        attention(pid, False, lambda: ffn_down(pid - 1, x1_s, 0, 0, T))
        z = attn_proj(pid)
        q_part()
        k_part(pid + 1)
        v_part(pid + 1)
        ln2(pid, z)
        ffn_up()
        k8_build(pid + 1)
        v_check(pid + 1)
        ln1(jnp.minimum(pid + 2, NBLK - 1))
        o_copy((pid - 1) * T, T, pid - 1).start()

    @pl.when(pid == NBLK - 1)
    def _():
        last = NBLK - 1
        attention(last, False, lambda: ffn_down(last - 1, x1_s, 0, 0, HT))
        z = attn_proj(last)
        x1c_s[...] = x1_s[HT:T, :]
        ffn_down(last - 1, x1c_s, 0, HT, T)
        o_copy((last - 1) * T, T, last - 1).start()
        ln2(last, z)
        ffn_up()
        tail = []
        for j, (lo, hi) in enumerate(zip(LASTCUT[:-1], LASTCUT[1:])):
            ffn_down(last, x1_s, lo, lo, hi)
            tail.append(o_copy(last * T + lo, hi - lo, last + j))
            tail[-1].start()
        v_bad = fold(vflag_s[...].reshape(NBLK * 8, 128), jnp.maximum)
        any_bad = jnp.max(
            jnp.maximum(fold(flag_s[...].reshape(NBLK * 8, 128), jnp.maximum), v_bad))
        for i in range(last):
            o_copy(i * T, T, i).wait()
        for cpy in tail:
            cpy.wait()

        @pl.when(any_bad > 0)
        def _():
            @pl.when(jnp.max(jnp.maximum(flag_s[0], v_bad)) > 0)
            def _():
                redo(0, True)

            def one(blk, carry):
                @pl.when(jnp.max(jnp.maximum(flag_s[blk], v_bad)) > 0)
                def _():
                    redo(blk, False)

                return carry

            jax.lax.fori_loop(1, NBLK, one, 0)


@jax.jit
def pallas_adaLN_cond__sliding_block__dense_activation_relu__prompt_kernel(
    A_x: jax.Array,
    A_wqkv: jax.Array,
    A_wo: jax.Array,
    B_x: jax.Array,
    B_w1: jax.Array,
    B_w2: jax.Array,
    c: jax.Array,
    w_mod: jax.Array,
):
    del B_x
    x = A_x.reshape(S, D)
    any_spec = pl.BlockSpec(memory_space=pl.ANY)
    scratch = [
        pltpu.VMEM((S, D), BF),
        pltpu.VMEM((D, D), BF),
        pltpu.VMEM((D, D), BF),
        pltpu.VMEM((D, D), BF),
        pltpu.VMEM((D, D), BF),
        pltpu.VMEM((D, DFF), BF),
        pltpu.VMEM((DFF, D), BF),
        pltpu.VMEM((1, D), BF),
        pltpu.VMEM((D, 6 * D), BF),
        pltpu.VMEM((D, D), BF),
        pltpu.VMEM((D, D), BF),
        pltpu.VMEM((8, 6 * D), F32),
        pltpu.VMEM((T, D), BF),
        pltpu.VMEM((HT, D), U32),
        pltpu.VMEM((T, D), BF),
        pltpu.VMEM((HT, D), U32),
        pltpu.VMEM((S // 2 + 64, D), U32),
        pltpu.VMEM((H, S // 2, 128), U32),
        pltpu.VMEM((S // 128, D // 2, 128), U32),
        pltpu.VMEM((D // 2, T), U32),
        pltpu.VMEM((D, T), F32),
        pltpu.VMEM((H, T), F32),
        pltpu.VMEM((T, D), F32),
        pltpu.VMEM((T, D), BF),
        pltpu.VMEM((HT, D), F32),
        pltpu.VMEM((T, DFF), BF),
        pltpu.VMEM((S, D), BF),
        pltpu.VMEM((T, D), BF),
        pltpu.VMEM((D // 2, T), U32),
        pltpu.VMEM((NBLK, 8, 128), jnp.int32),
        pltpu.VMEM((NBLK, 8, 128), jnp.int32),
        pltpu.SemaphoreType.DMA((NSEM,)),
    ]
    out = pl.pallas_call(
        _kernel,
        grid=(NBLK,),
        in_specs=[any_spec] * 7,
        out_specs=any_spec,
        out_shape=jax.ShapeDtypeStruct((S, D), BF),
        scratch_shapes=scratch,
        compiler_params=pltpu.CompilerParams(
            dimension_semantics=("arbitrary",),
            vmem_limit_bytes=100 * 1024 * 1024),
    )(x, A_wqkv, A_wo, B_w1, B_w2, c, w_mod)
    return out.reshape(1, S, D)
```

```python
import jax
import jax.numpy as jnp
import jax.experimental.pallas as pl
import jax.experimental.pallas.tpu as pltpu

F32 = jnp.float32
BF = jnp.bfloat16
U32 = jnp.uint32

S = 2048
D = 512
H = 32
DFF = 1792
T = 256
HT = T // 2
HD = D // 2
NBLK = S // T
EPS = 1e-5
QSCALE = 0.25 * 1.4426950408889634
NEG = -1e30
NT = (((1,), (1,)), ((), ()))

LNR = 16
L_LO_BITS, L_HI_BITS = (127 - 50) << 23, (127 + 100) << 23
V_LO_BITS, V_HI_BITS = (127 - 40) << 23, (127 + 20) << 23
QK_CUTS = (0, 64, 128, 192, 272)
CUTS0 = (144, 208, 272)
CUTS1 = (16, 80, 144, 208, 272)
DA = 2
DB = 1
DA0 = 5
DB0 = 3
LASTCUT = (0, 128, 192, 256)

(SEM_C, SEM_WMA, SEM_WQ, SEM_WV, SEM_WKA, SEM_WKB, SEM_WMB, SEM_WO, SEM_W1, SEM_W2,
 SEM_WMC) = range(11)
SEM_X0 = 11
SEM_O0 = SEM_X0 + NBLK
NSEM = SEM_O0 + NBLK - 1 + len(LASTCUT) - 1


def _u32(x):
    return x if x.dtype == U32 else pltpu.bitcast(x, U32)


def _pack_pairs(a, b):
    return _u32(pltpu.pack_elementwise([a, b], packed_dtype=BF))


def _layernorm(x):
    mu = jnp.mean(x, axis=-1, keepdims=True)
    xc = x - mu
    var = jnp.mean(xc * xc, axis=-1, keepdims=True)
    return xc * jax.lax.rsqrt(var + EPS)


def _kernel(x_hbm, wqkv_hbm, wo_hbm, w1_hbm, w2_hbm, c_hbm, wmod_hbm, out_hbm,
            x_v, wq_v, wk_v, wv_v, wo_v, w1_v, w2_v, c_v, wmod_v,
            wqt_s, wvt_s, mod_s, hn_s, hp_s, hn0_s, hp0_s, k_s, k8_s, vt_s, qt_s, ot_s, l_s,
            x1_s, h2_s, x1c_s, a_s, o_s, hf_s, qf_s, flag_s, vflag_s, sems):
    pid = pl.program_id(0)

    def cp(src, dst, slot):
        return pltpu.make_async_copy(src, dst, sems.at[slot])

    def x_copy(i):
        return cp(x_hbm.at[pl.ds(i * T, T), :], x_v.at[pl.ds(i * T, T), :], SEM_X0 + i)

    def o_copy(r0, n, slot):
        return cp(o_s.at[pl.ds(r0, n), :], out_hbm.at[pl.ds(r0, n), :], SEM_O0 + slot)

    c_copy = cp(c_hbm, c_v, SEM_C)
    wma_copy = cp(wmod_hbm.at[:, pl.ds(0, 2 * D)], wmod_v.at[:, pl.ds(0, 2 * D)], SEM_WMA)
    wmb_copy = cp(wmod_hbm.at[:, pl.ds(2 * D, 3 * D)], wmod_v.at[:, pl.ds(2 * D, 3 * D)], SEM_WMB)
    wmc_copy = cp(wmod_hbm.at[:, pl.ds(5 * D, D)], wmod_v.at[:, pl.ds(5 * D, D)], SEM_WMC)
    wq_copy = cp(wqkv_hbm.at[:, pl.ds(0, D)], wq_v, SEM_WQ)
    wka_copy = cp(wqkv_hbm.at[:, pl.ds(D, HD)], wk_v.at[:, pl.ds(0, HD)], SEM_WKA)
    wkb_copy = cp(wqkv_hbm.at[:, pl.ds(D + HD, HD)], wk_v.at[:, pl.ds(HD, HD)], SEM_WKB)
    wv_copy = cp(wqkv_hbm.at[:, pl.ds(2 * D, D)], wv_v, SEM_WV)
    wo_copy = cp(wo_hbm, wo_v, SEM_WO)
    w1_copy = cp(w1_hbm, w1_v, SEM_W1)
    w2_copy = cp(w2_hbm, w2_v, SEM_W2)

    def mod_part(lo, hi):
        cf = c_v[...].astype(F32)
        sc = cf * (1.0 / (1.0 + jnp.exp(-cf)))
        sc = jnp.broadcast_to(sc, (16, D)).astype(BF)
        m = jnp.dot(sc, wmod_v[:, lo:hi], preferred_element_type=F32)
        mod_s[:, lo:hi] = m[0:8]

    def modrow(k):
        return mod_s[0:1, k * D:(k + 1) * D]

    def ln1_pre():
        for r in range(0, T, LNR):
            x1_s[r:r + LNR, :] = _layernorm(x_v[r:r + LNR, :].astype(F32))

    def ln1(blk, hn_s=hn_s, hp_s=hp_s, pre=False):
        r0 = pl.multiple_of(blk * T, T)
        g1 = 1.0 + modrow(1)
        sh = modrow(0)
        for r in range(0, T, LNR):
            if pre:
                xn = x1_s[r:r + LNR, :]
            else:
                xn = _layernorm(x_v[pl.ds(r0 + r, LNR), :].astype(F32))
            h = xn * g1 + sh
            hn_s[r:r + LNR, :] = h.astype(BF)
            for g in range(LNR // 16):
                hp_s[r // 2 + 8 * g:r // 2 + 8 * g + 8, :] = _pack_pairs(
                    h[16 * g:16 * g + 8], h[16 * g + 8:16 * g + 16])

    def q_part(hn_s=hn_s):
        qt = jax.lax.dot_general(wqt_s[...], hn_s[...], NT, preferred_element_type=F32) * QSCALE
        qt_s[...] = _u32(qt.astype(BF))

    def k_part(blk, hn_s=hn_s, lo=0, hi=D):
        k = jnp.dot(hn_s[...], wk_v[:, lo:hi], preferred_element_type=F32)
        r0 = pl.multiple_of(blk * HT + 64, 64)
        k_s[pl.ds(r0, HT), lo:hi] = _u32(k.astype(BF))

    def v_part(blk, hp_s=hp_s):
        hp = pltpu.bitcast(hp_s[...], BF)
        vt = jax.lax.dot_general(wvt_s[...], hp, NT, preferred_element_type=F32)
        for b in range(T // 128):
            vt_s[blk * (T // 128) + b] = _u32(vt[:, 128 * b:128 * b + 128].astype(BF))

    def fold(x, op):
        t = [x[r:r + 8, c:c + 128] for r in range(0, x.shape[0], 8)
             for c in range(0, x.shape[1], 128)]
        while len(t) > 1:
            t = [op(t[i], t[i + 1]) for i in range(0, len(t), 2)]
        return t[0]

    def v_check(blk):
        mn = mx = None
        for b in range(T // 128):
            for r in range(0, D // 2, 8):
                u = pltpu.bitcast(vt_s[blk * (T // 128) + b, r:r + 8, :], jnp.int32)
                for m in (u & 0x7FFF0000, (u << 16) & 0x7FFF0000):
                    nz = (m - 0x10000) & 0x7FFF0000
                    mn = nz if mn is None else jnp.minimum(mn, nz)
                    mx = m if mx is None else jnp.maximum(mx, m)
        bad = (mn < V_LO_BITS) | (mx > V_HI_BITS)
        vflag_s[blk] = jnp.where(bad, 1, 0)

    def k8_build(blk):
        lane = jax.lax.broadcasted_iota(jnp.int32, (8, 128), 1)
        bit = [((lane >> (4 + k)) & 1) == 1 for k in range(3)]
        src0 = blk * HT + 8
        dst0 = blk * HT
        for g in range(4):
            xs = {}

            def x(w, g=g, xs=xs):
                if w not in xs:
                    xs[w] = k_s[pl.ds(pl.multiple_of(src0 + 8 * w, 8), 8), 128 * g:128 * g + 128]
                return xs[w]

            for u in range(T // 16):
                f = [x(u)] + [pltpu.roll(x(u + d), 16 * d, 1) for d in range(1, 8)]
                for k in range(3):
                    f = [jnp.where(bit[k], f[(m + (1 << k)) % 8], f[m]) for m in range(8)]
                for hh in range(8):
                    k8_s[8 * g + hh, pl.ds(pl.multiple_of(dst0 + 8 * u, 8), 8), :] = f[(-hh) % 8]

    def attention(blk, first, filler=None, safe=False):
        lane8 = jax.lax.broadcasted_iota(jnp.int32, (8, 128), 1)
        srow = jax.lax.broadcasted_iota(jnp.int32, (8, 128), 0)
        i16 = lane8 & 15
        first_m = [8 * v + srow > i16 for v in range(2)]
        last_m = [8 * v + srow <= i16 for v in range(2)]
        blkid = lane8 >> 4
        blkge = [blkid >= s for s in range(8)]
        bit = [((blkid >> k) & 1) == 1 for k in range(3)]
        zero8 = jnp.zeros((8, 128), U32)
        neg8 = jnp.full((8, 128), NEG, F32)

        def rows(h, n):
            return pl.ds(pl.multiple_of(n * h, n), n)

        def qk(b, h):
            nneg = max(0, 256 - 128 * b) if first else 0
            tmin = max(0, nneg - 112)
            cuts = QK_CUTS if tmin == 0 else (CUTS1 if tmin == 16 else CUTS0)
            if safe:
                qv = qf_s[rows(h, 8), 128 * b:128 * b + 128]
                parts = [jnp.where(blkid == ((s - h) & 7), qv, zero8) for s in range(8)]
                cuts = (cuts[0], cuts[-1])
            else:
                lvl = [qt_s[8 * h:8 * h + 8, 128 * b:128 * b + 128]]
                for k in (2, 1, 0):
                    lvl = [x for y in lvl
                           for x in (jnp.where(bit[k], zero8, y), jnp.where(bit[k], y, zero8))]
                parts = [lvl[(s - h) % 8] for s in range(8)]
            w = pltpu.bitcast(jnp.concatenate(parts, axis=0), BF)
            sv = {}
            row0 = blk * HT + 64 * b - 72
            for a_, b_ in zip(cuts[:-1], cuts[1:]):
                kc = k8_s[h, pl.ds(pl.multiple_of(row0 + a_ // 2, 8), (b_ - a_) // 2), :]
                sc = jnp.dot(pltpu.bitcast(kc, BF), w, preferred_element_type=F32)
                for v in range((b_ - a_) // 8):
                    sv[a_ // 8 + v] = sc[8 * v:8 * v + 8]
            return sv, nneg

        def mask_max(sv, nneg):
            for v in sorted(sv):
                if v < 2:
                    sv[v] = jnp.where(first_m[v], sv[v], neg8)
                elif v >= 32:
                    sv[v] = jnp.where(last_m[v - 32], sv[v], neg8)
                if 8 * v < nneg:
                    smin = -((8 * v - nneg) // 16)
                    sv[v] = jnp.where(blkge[smin], sv[v], neg8)
            if not safe:
                return None, sv
            vs = sorted(sv)
            m0, m1 = sv[vs[0]], sv[vs[1]]
            for v in vs[2::2]:
                m0 = jnp.maximum(m0, sv[v])
                m1 = jnp.maximum(m1, sv[v + 1])
            m = jnp.max(jnp.maximum(m0, m1), axis=0, keepdims=True)
            return jnp.broadcast_to(m, (8, 128)), sv

        def probs(b, h, st):
            m, sv = st
            c0 = max(0, 2 - b) if first else 0
            lv = [{}, {}, {}]
            outv = []

            def sel(mk, a, c):
                if a is None and c is None:
                    return None
                return jnp.where(mk, zero8 if a is None else a, zero8 if c is None else c)

            l0 = l1 = None
            for v in range(24):
                if v < 17 and 2 * v in sv:
                    a = jnp.exp2(sv[2 * v] - m if safe else sv[2 * v])
                    c = jnp.exp2(sv[2 * v + 1] - m if safe else sv[2 * v + 1])
                    l0 = a if l0 is None else l0 + a
                    l1 = c if l1 is None else l1 + c
                    lv[0][v] = _pack_pairs(a, c)
                if v < 18:
                    lv[1][v] = sel(bit[0], lv[0].get(v - 1), lv[0].get(v))
                if v < 20:
                    lv[2][v] = sel(bit[1], lv[1].get(v - 2), lv[1].get(v))
                if v >= 8 * c0:
                    o = sel(bit[2], lv[2].get(v - 4), lv[2].get(v))
                    outv.append(zero8 if o is None else o)
            l = jnp.sum(l0 + l1, axis=0, keepdims=True)
            if safe:
                return outv, l
            l_s[h:h + 1, 128 * b:128 * b + 128] = l
            return outv, None

        def pv(b, h, st):
            outv, l = st
            c0 = max(0, 2 - b) if first else 0
            tile0 = blk * (T // 128) + b - 2
            acc = None
            for c in range(c0, 3):
                pt = pltpu.bitcast(
                    jnp.concatenate(outv[8 * (c - c0):8 * (c - c0) + 8], axis=0), BF)
                vt = vt_s[tile0 + c, rows(h, 8), :]
                o = jnp.dot(pltpu.bitcast(vt, BF), pt, preferred_element_type=F32)
                acc = o if acc is None else acc + o
            if safe:
                acc = acc * (1.0 / l)
            ot_s[rows(h, 16), 128 * b:128 * b + 128] = acc

        if safe:
            for b in range(T // 128):
                def head(h, carry, b=b):
                    pv(b, h, probs(b, h, mask_max(*qk(b, h))))
                    return carry

                jax.lax.fori_loop(0, H, head, 0)
            return

        items = [(b, h) for b in range(T // 128) for h in range(H)]
        n = len(items)
        sa, sb = {}, {}
        da, db = (DA0, DB0) if first else (DA, DB)
        for t in range(n + da + db):
            st = qk(*items[t]) if t < n else None
            if 0 <= t - da < n:
                sb[t - da] = probs(*items[t - da], sa.pop(t - da))
            if 0 <= t - da - db < n:
                pv(*items[t - da - db], sb.pop(t - da - db))
            if st is not None:
                sa[t] = mask_max(*st)
            if filler is not None and t == n:
                filler()

    def attn_proj(blk):
        l = l_s[...]
        rl = 1.0 / l
        parts = [ot_s[16 * h:16 * h + 16, :] * rl[h:h + 1, :] for h in range(H)]
        li = pltpu.bitcast(l, jnp.int32)
        bad = (fold(li, jnp.minimum) < L_LO_BITS) | (fold(li, jnp.maximum) > L_HI_BITS)
        flag_s[blk] = jnp.where(bad, 1, 0)
        o = jnp.concatenate(parts, axis=0).T.astype(BF)
        return jnp.dot(o, wo_v[...], preferred_element_type=F32)

    def ln2(blk, z):
        r0 = pl.multiple_of(blk * T, T)
        g2 = 1.0 + modrow(4)
        sh = modrow(3)
        ga = modrow(2)
        for r in range(0, T, LNR):
            x1 = x_v[pl.ds(r0 + r, LNR), :].astype(F32) + ga * z[r:r + LNR]
            x1_s[r:r + LNR, :] = x1
            h2 = _layernorm(x1) * g2 + sh
            h2_s[r:r + LNR, :] = h2.astype(BF)

    def ffn_up():
        a = jnp.dot(h2_s[...], w1_v[...], preferred_element_type=F32)
        a_s[...] = jnp.maximum(a, 0.0).astype(BF)

    def ffn_down(blk, res_ref, rlo, lo, hi):
        y = jnp.dot(a_s[lo:hi, :], w2_v[...], preferred_element_type=F32)
        r0 = pl.multiple_of(blk * T + lo, 64)
        o_s[pl.ds(r0, hi - lo), :] = (
            res_ref[rlo:rlo + hi - lo, :] + modrow(5) * y).astype(BF)

    def redo(blk, first):
        r0 = pl.multiple_of(blk * T, T)
        g1 = 1.0 + modrow(1)
        sh1 = modrow(0)

        def ln_rows(i, carry):
            r = pl.multiple_of(i * 16, 16)
            xn = _layernorm(x_v[pl.ds(pl.multiple_of(r0 + r, 16), 16), :].astype(F32))
            hf_s[pl.ds(r, 16), :] = (xn * g1 + sh1).astype(BF)
            return carry

        jax.lax.fori_loop(0, T // 16, ln_rows, 0)

        def q_rows(j, carry):
            wt = wqt_s[pl.ds(pl.multiple_of(j * 128, 128), 128), :]
            qt = jax.lax.dot_general(wt, hf_s[...], NT, preferred_element_type=F32) * QSCALE
            qf_s[pl.ds(pl.multiple_of(j * 64, 64), 64), :] = _u32(qt.astype(BF))
            return carry

        jax.lax.fori_loop(0, D // 128, q_rows, 0)
        attention(blk, first, safe=True)
        hf_s[...] = ot_s[...].T.astype(BF)
        g2 = 1.0 + modrow(4)
        sh2 = modrow(3)
        ga = modrow(2)
        gb = modrow(5)

        def tail_rows(i, carry):
            r = pl.multiple_of(i * 32, 32)
            rows = pl.ds(pl.multiple_of(r0 + r, 32), 32)
            z = jnp.dot(hf_s[pl.ds(r, 32), :], wo_v[...], preferred_element_type=F32)
            x1 = x_v[rows, :].astype(F32) + ga * z
            h2 = (_layernorm(x1) * g2 + sh2).astype(BF)
            a = jnp.dot(h2, w1_v[...], preferred_element_type=F32)
            a = jnp.maximum(a, 0.0).astype(BF)
            y = jnp.dot(a, w2_v[...], preferred_element_type=F32)
            o_s[rows, :] = (x1 + gb * y).astype(BF)
            return carry

        jax.lax.fori_loop(0, T // 32, tail_rows, 0)
        cpy = o_copy(r0, T, 0)
        cpy.start()
        cpy.wait()

    def first_step():
        for cpy in (c_copy, x_copy(0), wma_copy, wka_copy, x_copy(1), wkb_copy, wq_copy, wv_copy,
                    wo_copy, wmb_copy, w1_copy, x_copy(2), wmc_copy, w2_copy):
            cpy.start()
        for i in range(3, NBLK):
            x_copy(i).start()
        k_s[0:64, :] = jnp.zeros((64, D), U32)
        c_copy.wait()
        x_copy(0).wait()
        ln1_pre()
        wma_copy.wait()
        mod_part(0, 2 * D)
        ln1(0, hn0_s, hp0_s, True)
        wka_copy.wait()
        k_part(0, hn0_s, 0, HD)
        x_copy(1).wait()
        wkb_copy.wait()
        k_part(0, hn0_s, HD, D)
        ln1(1)
        wq_copy.wait()
        k_part(1)
        wqt_s[...] = wq_v[...].T
        wv_copy.wait()
        q_part(hn0_s)
        wvt_s[...] = wv_v[...].T
        k8_build(0)
        v_part(0, hp0_s)
        v_part(1)
        v_check(0)
        v_check(1)
        attention(0, True)
        wo_copy.wait()
        wmb_copy.wait()
        mod_part(2 * D, 5 * D)
        z = attn_proj(0)
        q_part()
        k8_build(1)
        ln2(0, z)
        wmc_copy.wait()
        w1_copy.wait()
        x_copy(2).wait()
        ln1(2)
        ffn_up()
        mod_part(5 * D, 6 * D)
        w2_copy.wait()
        x_copy(3).wait()

    def middle_step():
        attention(pid, False, lambda: ffn_down(pid - 1, x1_s, 0, 0, T))
        z = attn_proj(pid)
        q_part()
        k_part(pid + 1)
        v_part(pid + 1)
        ln2(pid, z)
        ffn_up()
        k8_build(pid + 1)
        v_check(pid + 1)
        ln1(jnp.minimum(pid + 2, NBLK - 1))
        o_copy((pid - 1) * T, T, pid - 1).start()

    def last_step():
        last = NBLK - 1
        attention(last, False, lambda: ffn_down(last - 1, x1_s, 0, 0, HT))
        z = attn_proj(last)
        x1c_s[...] = x1_s[HT:T, :]
        ffn_down(last - 1, x1c_s, 0, HT, T)
        o_copy((last - 1) * T, T, last - 1).start()
        ln2(last, z)
        ffn_up()
        tail = []
        for j, (lo, hi) in enumerate(zip(LASTCUT[:-1], LASTCUT[1:])):
            ffn_down(last, x1_s, lo, lo, hi)
            tail.append(o_copy(last * T + lo, hi - lo, last + j))
            tail[-1].start()
        v_bad = fold(vflag_s[...].reshape(NBLK * 8, 128), jnp.maximum)
        any_bad = jnp.max(
            jnp.maximum(fold(flag_s[...].reshape(NBLK * 8, 128), jnp.maximum), v_bad))
        for i in range(last):
            o_copy(i * T, T, i).wait()
        for cpy in tail:
            cpy.wait()

        @pl.when(any_bad > 0)
        def _():
            @pl.when(jnp.max(jnp.maximum(flag_s[0], v_bad)) > 0)
            def _():
                redo(0, True)

            def one(blk, carry):
                @pl.when(jnp.max(jnp.maximum(flag_s[blk], v_bad)) > 0)
                def _():
                    redo(blk, False)

                return carry

            jax.lax.fori_loop(1, NBLK, one, 0)

    def inner_step():
        middle_step()

        @pl.when(pid == 1)
        def _():
            for i in range(4, NBLK):
                x_copy(i).wait()

    def outer_step():
        jax.lax.cond(pid == 0, first_step, last_step)

    jax.lax.cond((pid > 0) & (pid < NBLK - 1), inner_step, outer_step)


@jax.jit
def pallas_adaLN_cond__sliding_block__dense_activation_relu__prompt_kernel(
    A_x: jax.Array,
    A_wqkv: jax.Array,
    A_wo: jax.Array,
    B_x: jax.Array,
    B_w1: jax.Array,
    B_w2: jax.Array,
    c: jax.Array,
    w_mod: jax.Array,
):
    del B_x
    x = A_x.reshape(S, D)
    any_spec = pl.BlockSpec(memory_space=pl.ANY)
    scratch = [
        pltpu.VMEM((S, D), BF),
        pltpu.VMEM((D, D), BF),
        pltpu.VMEM((D, D), BF),
        pltpu.VMEM((D, D), BF),
        pltpu.VMEM((D, D), BF),
        pltpu.VMEM((D, DFF), BF),
        pltpu.VMEM((DFF, D), BF),
        pltpu.VMEM((1, D), BF),
        pltpu.VMEM((D, 6 * D), BF),
        pltpu.VMEM((D, D), BF),
        pltpu.VMEM((D, D), BF),
        pltpu.VMEM((8, 6 * D), F32),
        pltpu.VMEM((T, D), BF),
        pltpu.VMEM((HT, D), U32),
        pltpu.VMEM((T, D), BF),
        pltpu.VMEM((HT, D), U32),
        pltpu.VMEM((S // 2 + 64, D), U32),
        pltpu.VMEM((H, S // 2, 128), U32),
        pltpu.VMEM((S // 128, D // 2, 128), U32),
        pltpu.VMEM((D // 2, T), U32),
        pltpu.VMEM((D, T), F32),
        pltpu.VMEM((H, T), F32),
        pltpu.VMEM((T, D), F32),
        pltpu.VMEM((T, D), BF),
        pltpu.VMEM((HT, D), F32),
        pltpu.VMEM((T, DFF), BF),
        pltpu.VMEM((S, D), BF),
        pltpu.VMEM((T, D), BF),
        pltpu.VMEM((D // 2, T), U32),
        pltpu.VMEM((NBLK, 8, 128), jnp.int32),
        pltpu.VMEM((NBLK, 8, 128), jnp.int32),
        pltpu.SemaphoreType.DMA((NSEM,)),
    ]
    out = pl.pallas_call(
        _kernel,
        grid=(NBLK,),
        in_specs=[any_spec] * 7,
        out_specs=any_spec,
        out_shape=jax.ShapeDtypeStruct((S, D), BF),
        scratch_shapes=scratch,
        compiler_params=pltpu.CompilerParams(
            dimension_semantics=("arbitrary",),
            vmem_limit_bytes=100 * 1024 * 1024),
    )(x, A_wqkv, A_wo, B_w1, B_w2, c, w_mod)
    return out.reshape(1, S, D)
```

```python
import jax
import jax.numpy as jnp
import jax.experimental.pallas as pl
import jax.experimental.pallas.tpu as pltpu

F32 = jnp.float32
BF = jnp.bfloat16
U32 = jnp.uint32

S = 2048
D = 512
H = 32
DFF = 1792
T = 256
HT = T // 2
HD = D // 2
NBLK = S // T
EPS = 1e-5
QSCALE = 0.25 * 1.4426950408889634
NEG = -1e30
NT = (((1,), (1,)), ((), ()))

LNR = 16
L_LO_BITS, L_HI_BITS = (127 - 50) << 23, (127 + 100) << 23
V_LO_BITS, V_HI_BITS = (127 - 40) << 23, (127 + 20) << 23
QK_CUTS = (0, 64, 128, 192, 272)
CUTS0 = (144, 208, 272)
CUTS1 = (16, 80, 144, 208, 272)
DA = 2
DB = 1
DA0 = 5
DB0 = 3
LASTCUT = (0, 192, 256)

(SEM_C, SEM_WMA, SEM_WQ, SEM_WV, SEM_WKA, SEM_WKB, SEM_WMB, SEM_WO, SEM_W1, SEM_W2,
 SEM_WMC) = range(11)
SEM_X0 = 11
SEM_O0 = SEM_X0 + NBLK
NSEM = SEM_O0 + NBLK - 1 + len(LASTCUT) - 1


def _u32(x):
    return x if x.dtype == U32 else pltpu.bitcast(x, U32)


def _pack_pairs(a, b):
    return _u32(pltpu.pack_elementwise([a, b], packed_dtype=BF))


def _layernorm(x):
    mu = jnp.mean(x, axis=-1, keepdims=True)
    xc = x - mu
    var = jnp.mean(xc * xc, axis=-1, keepdims=True)
    return xc * jax.lax.rsqrt(var + EPS)


def _kernel(x_hbm, wqkv_hbm, wo_hbm, w1_hbm, w2_hbm, c_hbm, wmod_hbm, out_hbm,
            x_v, wq_v, wk_v, wv_v, wo_v, w1_v, w2_v, c_v, wmod_v,
            wqt_s, wvt_s, mod_s, hn_s, hp_s, hn0_s, hp0_s, k_s, k8_s, vt_s, qt_s, ot_s, l_s,
            x1_s, h2_s, x1c_s, a_s, o_s, hf_s, qf_s, flag_s, vflag_s, sems):
    pid = pl.program_id(0)

    def cp(src, dst, slot):
        return pltpu.make_async_copy(src, dst, sems.at[slot])

    def x_copy(i):
        return cp(x_hbm.at[pl.ds(i * T, T), :], x_v.at[pl.ds(i * T, T), :], SEM_X0 + i)

    def o_copy(r0, n, slot):
        return cp(o_s.at[pl.ds(r0, n), :], out_hbm.at[pl.ds(r0, n), :], SEM_O0 + slot)

    c_copy = cp(c_hbm, c_v, SEM_C)
    wma_copy = cp(wmod_hbm.at[:, pl.ds(0, 2 * D)], wmod_v.at[:, pl.ds(0, 2 * D)], SEM_WMA)
    wmb_copy = cp(wmod_hbm.at[:, pl.ds(2 * D, 3 * D)], wmod_v.at[:, pl.ds(2 * D, 3 * D)], SEM_WMB)
    wmc_copy = cp(wmod_hbm.at[:, pl.ds(5 * D, D)], wmod_v.at[:, pl.ds(5 * D, D)], SEM_WMC)
    wq_copy = cp(wqkv_hbm.at[:, pl.ds(0, D)], wq_v, SEM_WQ)
    wka_copy = cp(wqkv_hbm.at[:, pl.ds(D, HD)], wk_v.at[:, pl.ds(0, HD)], SEM_WKA)
    wkb_copy = cp(wqkv_hbm.at[:, pl.ds(D + HD, HD)], wk_v.at[:, pl.ds(HD, HD)], SEM_WKB)
    wv_copy = cp(wqkv_hbm.at[:, pl.ds(2 * D, D)], wv_v, SEM_WV)
    wo_copy = cp(wo_hbm, wo_v, SEM_WO)
    w1_copy = cp(w1_hbm, w1_v, SEM_W1)
    w2_copy = cp(w2_hbm, w2_v, SEM_W2)

    def mod_part(lo, hi):
        cf = c_v[...].astype(F32)
        sc = cf * (1.0 / (1.0 + jnp.exp(-cf)))
        sc = jnp.broadcast_to(sc, (16, D)).astype(BF)
        m = jnp.dot(sc, wmod_v[:, lo:hi], preferred_element_type=F32)
        mod_s[:, lo:hi] = m[0:8]

    def modrow(k):
        return mod_s[0:1, k * D:(k + 1) * D]

    def ln1_pre():
        for r in range(0, T, LNR):
            x1_s[r:r + LNR, :] = _layernorm(x_v[r:r + LNR, :].astype(F32))

    def ln1(blk, hn_s=hn_s, hp_s=hp_s, pre=False):
        r0 = pl.multiple_of(blk * T, T)
        g1 = 1.0 + modrow(1)
        sh = modrow(0)
        for r in range(0, T, LNR):
            if pre:
                xn = x1_s[r:r + LNR, :]
            else:
                xn = _layernorm(x_v[pl.ds(r0 + r, LNR), :].astype(F32))
            h = xn * g1 + sh
            hn_s[r:r + LNR, :] = h.astype(BF)
            for g in range(LNR // 16):
                hp_s[r // 2 + 8 * g:r // 2 + 8 * g + 8, :] = _pack_pairs(
                    h[16 * g:16 * g + 8], h[16 * g + 8:16 * g + 16])

    def q_part(hn_s=hn_s):
        qt = jax.lax.dot_general(wqt_s[...], hn_s[...], NT, preferred_element_type=F32) * QSCALE
        qt_s[...] = _u32(qt.astype(BF))

    def k_part(blk, hn_s=hn_s, lo=0, hi=D):
        k = jnp.dot(hn_s[...], wk_v[:, lo:hi], preferred_element_type=F32)
        r0 = pl.multiple_of(blk * HT + 64, 64)
        k_s[pl.ds(r0, HT), lo:hi] = _u32(k.astype(BF))

    def v_part(blk, hp_s=hp_s):
        hp = pltpu.bitcast(hp_s[...], BF)
        vt = jax.lax.dot_general(wvt_s[...], hp, NT, preferred_element_type=F32)
        for b in range(T // 128):
            vt_s[blk * (T // 128) + b] = _u32(vt[:, 128 * b:128 * b + 128].astype(BF))

    def fold(x, op):
        t = [x[r:r + 8, c:c + 128] for r in range(0, x.shape[0], 8)
             for c in range(0, x.shape[1], 128)]
        while len(t) > 1:
            t = [op(t[i], t[i + 1]) for i in range(0, len(t), 2)]
        return t[0]

    def v_check(blk):
        mn = mx = None
        for b in range(T // 128):
            for r in range(0, D // 2, 8):
                u = pltpu.bitcast(vt_s[blk * (T // 128) + b, r:r + 8, :], jnp.int32)
                for m in (u & 0x7FFF0000, (u << 16) & 0x7FFF0000):
                    nz = (m - 0x10000) & 0x7FFF0000
                    mn = nz if mn is None else jnp.minimum(mn, nz)
                    mx = m if mx is None else jnp.maximum(mx, m)
        bad = (mn < V_LO_BITS) | (mx > V_HI_BITS)
        vflag_s[blk] = jnp.where(bad, 1, 0)

    def k8_build(blk):
        lane = jax.lax.broadcasted_iota(jnp.int32, (8, 128), 1)
        bit = [((lane >> (4 + k)) & 1) == 1 for k in range(3)]
        src0 = blk * HT + 8
        dst0 = blk * HT
        for g in range(4):
            xs = {}

            def x(w, g=g, xs=xs):
                if w not in xs:
                    xs[w] = k_s[pl.ds(pl.multiple_of(src0 + 8 * w, 8), 8), 128 * g:128 * g + 128]
                return xs[w]

            for u in range(T // 16):
                f = [x(u)] + [pltpu.roll(x(u + d), 16 * d, 1) for d in range(1, 8)]
                for k in range(3):
                    f = [jnp.where(bit[k], f[(m + (1 << k)) % 8], f[m]) for m in range(8)]
                for hh in range(8):
                    k8_s[8 * g + hh, pl.ds(pl.multiple_of(dst0 + 8 * u, 8), 8), :] = f[(-hh) % 8]

    def attention(blk, first, filler=None, safe=False):
        lane8 = jax.lax.broadcasted_iota(jnp.int32, (8, 128), 1)
        srow = jax.lax.broadcasted_iota(jnp.int32, (8, 128), 0)
        i16 = lane8 & 15
        first_m = [8 * v + srow > i16 for v in range(2)]
        last_m = [8 * v + srow <= i16 for v in range(2)]
        blkid = lane8 >> 4
        blkge = [blkid >= s for s in range(8)]
        bit = [((blkid >> k) & 1) == 1 for k in range(3)]
        zero8 = jnp.zeros((8, 128), U32)
        neg8 = jnp.full((8, 128), NEG, F32)

        def rows(h, n):
            return pl.ds(pl.multiple_of(n * h, n), n)

        def qk(b, h):
            nneg = max(0, 256 - 128 * b) if first else 0
            tmin = max(0, nneg - 112)
            cuts = QK_CUTS if tmin == 0 else (CUTS1 if tmin == 16 else CUTS0)
            if safe:
                qv = qf_s[rows(h, 8), 128 * b:128 * b + 128]
                parts = [jnp.where(blkid == ((s - h) & 7), qv, zero8) for s in range(8)]
                cuts = (cuts[0], cuts[-1])
            else:
                lvl = [qt_s[8 * h:8 * h + 8, 128 * b:128 * b + 128]]
                for k in (2, 1, 0):
                    lvl = [x for y in lvl
                           for x in (jnp.where(bit[k], zero8, y), jnp.where(bit[k], y, zero8))]
                parts = [lvl[(s - h) % 8] for s in range(8)]
            w = pltpu.bitcast(jnp.concatenate(parts, axis=0), BF)
            sv = {}
            row0 = blk * HT + 64 * b - 72
            for a_, b_ in zip(cuts[:-1], cuts[1:]):
                kc = k8_s[h, pl.ds(pl.multiple_of(row0 + a_ // 2, 8), (b_ - a_) // 2), :]
                sc = jnp.dot(pltpu.bitcast(kc, BF), w, preferred_element_type=F32)
                for v in range((b_ - a_) // 8):
                    sv[a_ // 8 + v] = sc[8 * v:8 * v + 8]
            return sv, nneg

        def mask_max(sv, nneg):
            for v in sorted(sv):
                if v < 2:
                    sv[v] = jnp.where(first_m[v], sv[v], neg8)
                elif v >= 32:
                    sv[v] = jnp.where(last_m[v - 32], sv[v], neg8)
                if 8 * v < nneg:
                    smin = -((8 * v - nneg) // 16)
                    sv[v] = jnp.where(blkge[smin], sv[v], neg8)
            if not safe:
                return None, sv
            vs = sorted(sv)
            m0, m1 = sv[vs[0]], sv[vs[1]]
            for v in vs[2::2]:
                m0 = jnp.maximum(m0, sv[v])
                m1 = jnp.maximum(m1, sv[v + 1])
            m = jnp.max(jnp.maximum(m0, m1), axis=0, keepdims=True)
            return jnp.broadcast_to(m, (8, 128)), sv

        def probs(b, h, st):
            m, sv = st
            c0 = max(0, 2 - b) if first else 0
            lv = [{}, {}, {}]
            outv = []

            def sel(mk, a, c):
                if a is None and c is None:
                    return None
                return jnp.where(mk, zero8 if a is None else a, zero8 if c is None else c)

            l0 = l1 = None
            for v in range(24):
                if v < 17 and 2 * v in sv:
                    a = jnp.exp2(sv[2 * v] - m if safe else sv[2 * v])
                    c = jnp.exp2(sv[2 * v + 1] - m if safe else sv[2 * v + 1])
                    l0 = a if l0 is None else l0 + a
                    l1 = c if l1 is None else l1 + c
                    lv[0][v] = _pack_pairs(a, c)
                if v < 18:
                    lv[1][v] = sel(bit[0], lv[0].get(v - 1), lv[0].get(v))
                if v < 20:
                    lv[2][v] = sel(bit[1], lv[1].get(v - 2), lv[1].get(v))
                if v >= 8 * c0:
                    o = sel(bit[2], lv[2].get(v - 4), lv[2].get(v))
                    outv.append(zero8 if o is None else o)
            l = jnp.sum(l0 + l1, axis=0, keepdims=True)
            if safe:
                return outv, l
            l_s[h:h + 1, 128 * b:128 * b + 128] = l
            return outv, None

        def pv(b, h, st):
            outv, l = st
            c0 = max(0, 2 - b) if first else 0
            tile0 = blk * (T // 128) + b - 2
            acc = None
            for c in range(c0, 3):
                pt = pltpu.bitcast(
                    jnp.concatenate(outv[8 * (c - c0):8 * (c - c0) + 8], axis=0), BF)
                vt = vt_s[tile0 + c, rows(h, 8), :]
                o = jnp.dot(pltpu.bitcast(vt, BF), pt, preferred_element_type=F32)
                acc = o if acc is None else acc + o
            if safe:
                acc = acc * (1.0 / l)
            ot_s[rows(h, 16), 128 * b:128 * b + 128] = acc

        if safe:
            for b in range(T // 128):
                def head(h, carry, b=b):
                    pv(b, h, probs(b, h, mask_max(*qk(b, h))))
                    return carry

                jax.lax.fori_loop(0, H, head, 0)
            return

        items = [(b, h) for b in range(T // 128) for h in range(H)]
        n = len(items)
        sa, sb = {}, {}
        da, db = (DA0, DB0) if first else (DA, DB)
        for t in range(n + da + db):
            st = qk(*items[t]) if t < n else None
            if 0 <= t - da < n:
                sb[t - da] = probs(*items[t - da], sa.pop(t - da))
            if 0 <= t - da - db < n:
                pv(*items[t - da - db], sb.pop(t - da - db))
            if st is not None:
                sa[t] = mask_max(*st)
            if filler is not None and t == n:
                filler()

    def attn_proj(blk):
        l = l_s[...]
        rl = 1.0 / l
        parts = [ot_s[16 * h:16 * h + 16, :] * rl[h:h + 1, :] for h in range(H)]
        li = pltpu.bitcast(l, jnp.int32)
        bad = (fold(li, jnp.minimum) < L_LO_BITS) | (fold(li, jnp.maximum) > L_HI_BITS)
        flag_s[blk] = jnp.where(bad, 1, 0)
        o = jnp.concatenate(parts, axis=0).T.astype(BF)
        return jnp.dot(o, wo_v[...], preferred_element_type=F32)

    def ln2(blk, z):
        r0 = pl.multiple_of(blk * T, T)
        g2 = 1.0 + modrow(4)
        sh = modrow(3)
        ga = modrow(2)
        for r in range(0, T, LNR):
            x1 = x_v[pl.ds(r0 + r, LNR), :].astype(F32) + ga * z[r:r + LNR]
            x1_s[r:r + LNR, :] = x1
            h2 = _layernorm(x1) * g2 + sh
            h2_s[r:r + LNR, :] = h2.astype(BF)

    def ffn_up():
        a = jnp.dot(h2_s[...], w1_v[...], preferred_element_type=F32)
        a_s[...] = jnp.maximum(a, 0.0).astype(BF)

    def ffn_down(blk, res_ref, rlo, lo, hi):
        y = jnp.dot(a_s[lo:hi, :], w2_v[...], preferred_element_type=F32)
        r0 = pl.multiple_of(blk * T + lo, 64)
        o_s[pl.ds(r0, hi - lo), :] = (
            res_ref[rlo:rlo + hi - lo, :] + modrow(5) * y).astype(BF)

    def redo(blk, first):
        r0 = pl.multiple_of(blk * T, T)
        g1 = 1.0 + modrow(1)
        sh1 = modrow(0)

        def ln_rows(i, carry):
            r = pl.multiple_of(i * 16, 16)
            xn = _layernorm(x_v[pl.ds(pl.multiple_of(r0 + r, 16), 16), :].astype(F32))
            hf_s[pl.ds(r, 16), :] = (xn * g1 + sh1).astype(BF)
            return carry

        jax.lax.fori_loop(0, T // 16, ln_rows, 0)

        def q_rows(j, carry):
            wt = wqt_s[pl.ds(pl.multiple_of(j * 128, 128), 128), :]
            qt = jax.lax.dot_general(wt, hf_s[...], NT, preferred_element_type=F32) * QSCALE
            qf_s[pl.ds(pl.multiple_of(j * 64, 64), 64), :] = _u32(qt.astype(BF))
            return carry

        jax.lax.fori_loop(0, D // 128, q_rows, 0)
        attention(blk, first, safe=True)
        hf_s[...] = ot_s[...].T.astype(BF)
        g2 = 1.0 + modrow(4)
        sh2 = modrow(3)
        ga = modrow(2)
        gb = modrow(5)

        def tail_rows(i, carry):
            r = pl.multiple_of(i * 32, 32)
            rows = pl.ds(pl.multiple_of(r0 + r, 32), 32)
            z = jnp.dot(hf_s[pl.ds(r, 32), :], wo_v[...], preferred_element_type=F32)
            x1 = x_v[rows, :].astype(F32) + ga * z
            h2 = (_layernorm(x1) * g2 + sh2).astype(BF)
            a = jnp.dot(h2, w1_v[...], preferred_element_type=F32)
            a = jnp.maximum(a, 0.0).astype(BF)
            y = jnp.dot(a, w2_v[...], preferred_element_type=F32)
            o_s[rows, :] = (x1 + gb * y).astype(BF)
            return carry

        jax.lax.fori_loop(0, T // 32, tail_rows, 0)
        cpy = o_copy(r0, T, 0)
        cpy.start()
        cpy.wait()

    def first_step():
        for cpy in (c_copy, x_copy(0), wma_copy, wka_copy, x_copy(1), wkb_copy, wq_copy, wv_copy,
                    wo_copy, wmb_copy, w1_copy, x_copy(2), wmc_copy, w2_copy):
            cpy.start()
        for i in range(3, NBLK):
            x_copy(i).start()
        k_s[0:64, :] = jnp.zeros((64, D), U32)
        c_copy.wait()
        x_copy(0).wait()
        ln1_pre()
        wma_copy.wait()
        mod_part(0, 2 * D)
        ln1(0, hn0_s, hp0_s, True)
        wka_copy.wait()
        k_part(0, hn0_s, 0, HD)
        x_copy(1).wait()
        wkb_copy.wait()
        k_part(0, hn0_s, HD, D)
        ln1(1)
        wq_copy.wait()
        k_part(1)
        wqt_s[...] = wq_v[...].T
        wv_copy.wait()
        q_part(hn0_s)
        wvt_s[...] = wv_v[...].T
        k8_build(0)
        v_part(0, hp0_s)
        v_part(1)
        v_check(0)
        v_check(1)
        attention(0, True)
        wo_copy.wait()
        wmb_copy.wait()
        mod_part(2 * D, 5 * D)
        z = attn_proj(0)
        q_part()
        k8_build(1)
        ln2(0, z)
        wmc_copy.wait()
        w1_copy.wait()
        x_copy(2).wait()
        ln1(2)
        ffn_up()
        mod_part(5 * D, 6 * D)
        w2_copy.wait()
        x_copy(3).wait()

    def middle_step():
        attention(pid, False, lambda: ffn_down(pid - 1, x1_s, 0, 0, T))
        z = attn_proj(pid)
        q_part()
        k_part(pid + 1)
        v_part(pid + 1)
        ln2(pid, z)
        ffn_up()
        k8_build(pid + 1)
        v_check(pid + 1)
        ln1(jnp.minimum(pid + 2, NBLK - 1))

    def last_step():
        last = NBLK - 1
        o_copy(0, (last - 1) * T, 0).start()
        attention(last, False, lambda: ffn_down(last - 1, x1_s, 0, 0, HT))
        z = attn_proj(last)
        x1c_s[...] = x1_s[HT:T, :]
        ffn_down(last - 1, x1c_s, 0, HT, T)
        o_copy((last - 1) * T, T, last - 1).start()
        ln2(last, z)
        ffn_up()
        tail = []
        for j, (lo, hi) in enumerate(zip(LASTCUT[:-1], LASTCUT[1:])):
            ffn_down(last, x1_s, lo, lo, hi)
            tail.append(o_copy(last * T + lo, hi - lo, last + j))
            tail[-1].start()
        v_bad = fold(vflag_s[...].reshape(NBLK * 8, 128), jnp.maximum)
        any_bad = jnp.max(
            jnp.maximum(fold(flag_s[...].reshape(NBLK * 8, 128), jnp.maximum), v_bad))
        o_copy(0, (last - 1) * T, 0).wait()
        o_copy((last - 1) * T, T, last - 1).wait()
        for cpy in tail:
            cpy.wait()

        @pl.when(any_bad > 0)
        def _():
            @pl.when(jnp.max(jnp.maximum(flag_s[0], v_bad)) > 0)
            def _():
                redo(0, True)

            def one(blk, carry):
                @pl.when(jnp.max(jnp.maximum(flag_s[blk], v_bad)) > 0)
                def _():
                    redo(blk, False)

                return carry

            jax.lax.fori_loop(1, NBLK, one, 0)

    def inner_step():
        middle_step()

        @pl.when(pid == 1)
        def _():
            for i in range(4, NBLK):
                x_copy(i).wait()

    def outer_step():
        jax.lax.cond(pid == 0, first_step, last_step)

    jax.lax.cond((pid > 0) & (pid < NBLK - 1), inner_step, outer_step)


@jax.jit
def pallas_adaLN_cond__sliding_block__dense_activation_relu__prompt_kernel(
    A_x: jax.Array,
    A_wqkv: jax.Array,
    A_wo: jax.Array,
    B_x: jax.Array,
    B_w1: jax.Array,
    B_w2: jax.Array,
    c: jax.Array,
    w_mod: jax.Array,
):
    del B_x
    x = A_x.reshape(S, D)
    any_spec = pl.BlockSpec(memory_space=pl.ANY)
    scratch = [
        pltpu.VMEM((S, D), BF),
        pltpu.VMEM((D, D), BF),
        pltpu.VMEM((D, D), BF),
        pltpu.VMEM((D, D), BF),
        pltpu.VMEM((D, D), BF),
        pltpu.VMEM((D, DFF), BF),
        pltpu.VMEM((DFF, D), BF),
        pltpu.VMEM((1, D), BF),
        pltpu.VMEM((D, 6 * D), BF),
        pltpu.VMEM((D, D), BF),
        pltpu.VMEM((D, D), BF),
        pltpu.VMEM((8, 6 * D), F32),
        pltpu.VMEM((T, D), BF),
        pltpu.VMEM((HT, D), U32),
        pltpu.VMEM((T, D), BF),
        pltpu.VMEM((HT, D), U32),
        pltpu.VMEM((S // 2 + 64, D), U32),
        pltpu.VMEM((H, S // 2, 128), U32),
        pltpu.VMEM((S // 128, D // 2, 128), U32),
        pltpu.VMEM((D // 2, T), U32),
        pltpu.VMEM((D, T), F32),
        pltpu.VMEM((H, T), F32),
        pltpu.VMEM((T, D), F32),
        pltpu.VMEM((T, D), BF),
        pltpu.VMEM((HT, D), F32),
        pltpu.VMEM((T, DFF), BF),
        pltpu.VMEM((S, D), BF),
        pltpu.VMEM((T, D), BF),
        pltpu.VMEM((D // 2, T), U32),
        pltpu.VMEM((NBLK, 8, 128), jnp.int32),
        pltpu.VMEM((NBLK, 8, 128), jnp.int32),
        pltpu.SemaphoreType.DMA((NSEM,)),
    ]
    out = pl.pallas_call(
        _kernel,
        grid=(NBLK,),
        in_specs=[any_spec] * 7,
        out_specs=any_spec,
        out_shape=jax.ShapeDtypeStruct((S, D), BF),
        scratch_shapes=scratch,
        compiler_params=pltpu.CompilerParams(
            dimension_semantics=("arbitrary",),
            vmem_limit_bytes=100 * 1024 * 1024),
    )(x, A_wqkv, A_wo, B_w1, B_w2, c, w_mod)
    return out.reshape(1, S, D)
```
